```python
import jax
import jax.numpy as jnp

def _softmax(x, axis=-1):
    return jax.nn.softmax(x, axis=axis)
def _gelu(x):
    return jax.nn.gelu(x, approximate=True)
def _silu(x):
    return jax.nn.silu(x)
def _sigmoid(x):
    return jax.nn.sigmoid(x)
def _layernorm(x, axis=-1, eps=1e-5):
    m = jnp.mean(x, axis=axis, keepdims=True)
    v = jnp.var(x, axis=axis, keepdims=True)
    return (x - m) / jnp.sqrt(v + eps)
def _scatter_add(tgt, idx, src, axis=0):
    return tgt.at[idx].add(src)
def _segment_sum(src, seg, n):
    return jax.ops.segment_sum(src, seg, n)
class _Rng:
    def __init__(self, key):
        self._k = key
    def _next(self):
        self._k, sub = jax.random.split(self._k)
        return sub
    def normal(self, shape):
        return jax.random.normal(self._next(), shape, dtype=jnp.bfloat16)
    def randint(self, lo, hi, shape):
        return jax.random.randint(self._next(), shape, lo, hi, dtype=jnp.int32)
    def uniform(self, shape, lo=0.0, hi=1.0):
        return jax.random.uniform(self._next(), shape, jnp.bfloat16, lo, hi)
    def permutation(self, n):
        return jax.random.permutation(self._next(), n)


kernel_name = 'parallel_sum__sliding_block_cached__glu_gated_swiglu__decode'

def setup_inputs():
    _rng = _Rng(jax.random.key(int.from_bytes(__import__("os").urandom(4), "little")))
    _w = (lambda a: (lambda t: t.astype(jnp.bfloat16) if jnp.issubdtype(t.dtype, jnp.floating) else t)(jnp.asarray(a)))
    def _A_setup():
        B, Sq, D = 4, 1, 640
        Hq, Hkv, Sk, Dh = 32, 32, 8192, 192
        assert Hq % Hkv == 0, (Hq, Hkv)
        return {
            "x": _w((lambda *s: _rng.normal(s) * 0.05)(B, Sq, D)),
            "k_cache": _w((lambda *s: _rng.normal(s) * 0.05)(B, Hkv, Sk, Dh)),
            "v_cache": _w((lambda *s: _rng.normal(s) * 0.05)(B, Hkv, Sk, Dh)),
            "wq": _w((lambda *s: _rng.normal(s) * 0.05)(D, Hq * Dh) * (D ** -0.5)),
            "wo": _w((lambda *s: _rng.normal(s) * 0.05)(Hq * Dh, D) * ((Hq * Dh) ** -0.5)),
        }
    _A_in = _A_setup()

    def _B_setup():
        B, S, D, F = 4, 1, 640, 1536
        return {
            "x": _w((lambda *s: _rng.normal(s) * 0.05)(B, S, D)),
            "w1": _w((lambda *s: _rng.normal(s) * 0.05)(D, F) * (2.0 / D) ** 0.5),
            "w3": _w((lambda *s: _rng.normal(s) * 0.05)(D, F) * (2.0 / D) ** 0.5),
            "w2": _w((lambda *s: _rng.normal(s) * 0.05)(F, D) * (2.0 / F) ** 0.5),
        }
    _B_in = _B_setup()

    return {
        "A_x": _A_in["x"],
        "A_k_cache": _A_in["k_cache"],
        "A_v_cache": _A_in["v_cache"],
        "A_wq": _A_in["wq"],
        "A_wo": _A_in["wo"],
        "B_x": _B_in["x"],
        "B_w1": _B_in["w1"],
        "B_w3": _B_in["w3"],
        "B_w2": _B_in["w2"],
    }

def reference(A_x, A_k_cache, A_v_cache, A_wq, A_wo, B_x, B_w1, B_w3, B_w2):
    def _A_ref(x, k_cache, v_cache, wq, wo):
        B, Sq, D = x.shape
        Hq, Dh = 32, 192
        Hkv, Sk = k_cache.shape[1], k_cache.shape[2]
        W = min(4096, max(256, Sk // 4))
        rep = Hq // Hkv
        q = (lambda x, *d: x.transpose(*d))((x @ wq).reshape(B, Sq, Hq, Dh), 0, 2, 1, 3)
        k = jnp.repeat(k_cache[:, :, Sk - W:, :], rep, axis=1)
        v = jnp.repeat(v_cache[:, :, Sk - W:, :], rep, axis=1)
        scores = jnp.einsum("bhqd,bhkd->bhqk", q, k) * (Dh ** -0.5)
        p = _softmax(scores, axis=-1)
        o = jnp.einsum("bhqk,bhkd->bhqd", p, v)
        return (lambda x, *d: x.transpose(*d))(o, 0, 2, 1, 3).reshape(B, Sq, Hq * Dh) @ wo

    def _B_ref(x, w1, w3, w2):
        gate = jnp.einsum("bsd,df->bsf", x, w1)
        up = jnp.einsum("bsd,df->bsf", x, w3)
        h = _silu(gate) * up
        out = jnp.einsum("bsf,fd->bsd", h, w2)
        return out

    x = A_x
    xn = _layernorm(x, axis=-1)
    return x + _A_ref(xn, A_k_cache, A_v_cache, A_wq, A_wo) + _B_ref(xn, B_w1, B_w3, B_w2)
```

```python
import jax
import jax.numpy as jnp
from jax import lax
import jax.experimental.pallas as pl
import jax.experimental.pallas.tpu as pltpu

F32 = jnp.float32
BF16 = jnp.bfloat16

HQ = 32
DH = 192
HG = 4
GROWS = HG * DH
NA = 24
RA = 32
NJ = RA // 8
LANE = 128


def _kernel(x_hbm, k_hbm, v_hbm, wq_hbm, wo_hbm, w1_hbm, w3_hbm, w2_hbm,
            out_ref,
            x_v, wq_v, wo_v, w1_v, w3_v, w2_v, kbuf, vbuf, qblk, p_s, acc, ffn_s,
            wsem, ksem, vsem, *, B, D, S, W, F):
    NC = W // LANE
    NG = B * HQ // HG
    GPB = HQ // HG
    S0 = S - W

    def k_copy(g, j, c):
        slot = g % 2
        return pltpu.make_async_copy(
            k_hbm.at[pl.ds(g * NA, NA), pl.ds(j * 8, 8), pl.ds(S0 + c * LANE, LANE)],
            kbuf.at[slot, :, pl.ds(j * 8, 8), pl.ds(c * LANE, LANE)],
            ksem.at[slot])

    def v_copy(g, j, c):
        slot = (g % 2) * NJ + j
        return pltpu.make_async_copy(
            v_hbm.at[pl.ds(g * NA, NA), j, :, pl.ds(S0 + c * LANE, LANE)],
            vbuf.at[slot, :, :, pl.ds(c * LANE, LANE)],
            vsem.at[slot])

    def wait_all(buf, sem):
        pltpu.make_async_copy(buf, buf, sem).wait()

    def issue_pair(g, j):
        for c in range(NC):
            k_copy(g + 1, j, c).start(priority=0)
            v_copy(g, j, c).start(priority=1)

    def issue_v_alone(g, j):
        for c in range(NC):
            v_copy(g, j, c).start(priority=c % 2)

    def w_copy(src, dst, sem, j, c):
        cs = pl.ds(pl.multiple_of(c * LANE, LANE), LANE)
        return pltpu.make_async_copy(src.at[:, pl.ds(j * 8, 8), cs],
                                     dst.at[:, pl.ds(j * 8, 8), cs], sem)

    def loop(n, fn, unroll=1):
        def body(i, carry):
            fn(i)
            return carry
        lax.fori_loop(0, n, body, 0, unroll=unroll)

    def issue_wq(jj):
        def f(c):
            w_copy(wq_hbm, wq_v, wsem.at[1], jj, c).start(priority=0)
            w_copy(wq_hbm, wq_v, wsem.at[1], jj + 2, c).start(priority=1)
        loop(HQ * DH // LANE, f, unroll=4)

    def issue_w13(j):
        def f(c):
            w_copy(w1_hbm, w1_v, wsem.at[2], j, c).start(priority=0)
            w_copy(w3_hbm, w3_v, wsem.at[3], j, c).start(priority=1)
        loop(F // LANE, f, unroll=4)

    def issue_w2():
        for jj in range(4):
            for c in range(D // LANE):
                w_copy(w2_hbm, w2_v, wsem.at[4], jj, c).start(priority=0)
                w_copy(w2_hbm, w2_v, wsem.at[4], jj + 4, c).start(priority=1)

    def issue_k0(jj):
        for c in range(NC):
            k_copy(0, jj, c).start(priority=0)
            k_copy(0, jj + 2, c).start(priority=1)

    def issue_wo(lo, hi):
        def f(i):
            rg = lo + i
            for c in range(D // LANE):
                for p in range(2):
                    pltpu.make_async_copy(
                        wo_hbm.at[:, rg + 16 * p, :, pl.ds(c * LANE, LANE)],
                        wo_v.at[:, rg + 16 * p, :, pl.ds(c * LANE, LANE)],
                        wsem.at[5]).start(priority=p)
        loop(hi - lo, f)

    def qproj(xn, hg):
        w = wq_v[:, :, hg * GROWS:(hg + 1) * GROWS].reshape(D, GROWS)
        q = jnp.dot(xn, w, preferred_element_type=F32)
        q = q.astype(BF16).astype(F32)
        row = lax.broadcasted_iota(jnp.int32, (8, GROWS), 0)
        col = lax.broadcasted_iota(jnp.int32, (8, GROWS), 1)
        diag = (col >= row * DH) & (col < (row + 1) * DH)
        for b in range(B):
            qb = jnp.broadcast_to(q[b:b + 1, :], (8, GROWS))
            qblk[b * GPB + hg] = jnp.where(diag, qb, 0.0)

    def scores_softmax(g):
        slot = g % 2
        wait_all(kbuf.at[slot], ksem.at[slot])
        kk = kbuf[slot].reshape(GROWS, W)
        s = jnp.dot(qblk[g].astype(BF16), kk, preferred_element_type=F32)
        s = s * (DH ** -0.5)
        m = jnp.max(s, axis=-1, keepdims=True)
        e = jnp.exp(s - m)
        l = jnp.sum(e, axis=-1, keepdims=True)
        p_s[...] = e * (1.0 / l)

    def pv_wo(g, j):
        slot = (g % 2) * NJ + j
        wait_all(vbuf.at[slot], vsem.at[slot])
        b = g // GPB
        hg = g % GPB
        tot = acc[b]
        for hh in range(HG):
            pb = jnp.broadcast_to(p_s[hh:hh + 1, :], (8, W))
            for a in range(hh * (NA // HG), (hh + 1) * (NA // HG)):
                prod = vbuf[slot, a].astype(F32) * pb
                part = prod[:, 0:LANE]
                for c in range(1, NC):
                    part = part + prod[:, c * LANE:(c + 1) * LANE]
                o = jnp.sum(part, axis=-1, keepdims=True)
                wrow = wo_v[3 * hg + a // 8, 4 * (a % 8) + j].astype(F32)
                tot = tot + o * wrow
        acc[b] = tot

    xcp = pltpu.make_async_copy(x_hbm, x_v, wsem.at[0])
    xcp.start()
    issue_wq(0)
    xcp.wait()
    x = x_v[...].astype(F32)
    mu = jnp.mean(x, axis=-1, keepdims=True)
    xc = x - mu
    var = jnp.mean(xc * xc, axis=-1, keepdims=True)
    xn4 = xc / jnp.sqrt(var + 1e-5)
    xn = jnp.concatenate([xn4, jnp.zeros((8 - B, D), F32)], axis=0).astype(BF16)
    acc[...] = jnp.zeros(acc.shape, F32)
    issue_wq(1)
    for j in range(NJ):
        issue_w13(j)
    wait_all(wq_v, wsem.at[1])
    for hg in range(0, 3):
        qproj(xn, hg)
    issue_w2()
    for hg in range(3, 6):
        qproj(xn, hg)
    issue_k0(0)
    for hg in range(6, 8):
        qproj(xn, hg)
    issue_k0(1)
    wait_all(w1_v, wsem.at[2])
    wait_all(w3_v, wsem.at[3])
    gate = jnp.dot(xn, w1_v[...].reshape(D, F), preferred_element_type=F32)
    up = jnp.dot(xn, w3_v[...].reshape(D, F), preferred_element_type=F32)
    hmid = (gate * jax.nn.sigmoid(gate) * up).astype(BF16)
    issue_wo(0, 8)
    wait_all(w2_v, wsem.at[4])
    ffn_s[...] = jnp.dot(hmid, w2_v[...].reshape(F, D), preferred_element_type=F32)
    scores_softmax(0)
    issue_wo(8, 16)
    for j in range(NJ):
        issue_pair(0, j)
    wait_all(wo_v, wsem.at[5])

    def group_body(g, carry):
        for j in range(NJ):
            @pl.when(g < NG - 2)
            def _():
                issue_pair(g + 1, j)

            @pl.when(g == NG - 2)
            def _():
                issue_v_alone(g + 1, j)

            pv_wo(g, j)

        @pl.when(g < NG - 1)
        def _():
            scores_softmax(g + 1)
        return carry

    lax.fori_loop(0, NG, group_body, 0)

    attn = jnp.concatenate(
        [jnp.sum(acc[b], axis=0, keepdims=True) for b in range(B)], axis=0)
    res = x_v[...].astype(F32) + attn + ffn_s[0:B, :]
    out_ref[...] = res.astype(out_ref.dtype)


@jax.jit
def pallas_parallel_sum__sliding_block_cached__glu_gated_swiglu__decode_kernel(
    A_x: jax.Array,
    A_k_cache: jax.Array,
    A_v_cache: jax.Array,
    A_wq: jax.Array,
    A_wo: jax.Array,
    B_x: jax.Array,
    B_w1: jax.Array,
    B_w3: jax.Array,
    B_w2: jax.Array,
):
    B, Sq, D = A_x.shape
    _, Hkv, S, Dh = A_k_cache.shape
    F = B_w1.shape[1]
    assert Sq == 1 and Hkv == HQ and Dh == DH
    W = min(4096, max(256, S // 4))

    kt = jnp.swapaxes(A_k_cache, 2, 3).reshape(B * HQ * DH // RA, RA, S)
    vt = jnp.swapaxes(A_v_cache, 2, 3).reshape(B * HQ * DH // RA, NJ, 8, S)
    x2 = A_x.reshape(B, D)
    wq = A_wq.reshape(D // 32, 32, HQ * DH)
    wo = A_wo.reshape(24, HQ * DH // (24 * 8), 8, D)
    w1 = B_w1.reshape(D // 32, 32, F)
    w3 = B_w3.reshape(D // 32, 32, F)
    w2 = B_w2.reshape(24, F // 24, D)

    NG = B * HQ // HG
    kern = lambda *refs: _kernel(*refs, B=B, D=D, S=S, W=W, F=F)
    out = pl.pallas_call(
        kern,
        in_specs=[pl.BlockSpec(memory_space=pl.ANY)] * 8,
        out_specs=pl.BlockSpec(memory_space=pltpu.VMEM),
        out_shape=jax.ShapeDtypeStruct((B, D), A_x.dtype),
        scratch_shapes=[
            pltpu.VMEM((B, D), BF16),
            pltpu.VMEM(wq.shape, BF16),
            pltpu.VMEM(wo.shape, BF16),
            pltpu.VMEM(w1.shape, BF16),
            pltpu.VMEM(w3.shape, BF16),
            pltpu.VMEM(w2.shape, BF16),
            pltpu.VMEM((2, NA, RA, W), BF16),
            pltpu.VMEM((2 * NJ, NA, 8, W), BF16),
            pltpu.VMEM((NG, 8, GROWS), F32),
            pltpu.VMEM((8, W), F32),
            pltpu.VMEM((B, 8, D), F32),
            pltpu.VMEM((8, D), F32),
            pltpu.SemaphoreType.DMA((6,)),
            pltpu.SemaphoreType.DMA((2,)),
            pltpu.SemaphoreType.DMA((2 * NJ,)),
        ],
        compiler_params=pltpu.CompilerParams(vmem_limit_bytes=100 * 1024 * 1024),
    )(x2, kt, vt, wq, wo, w1, w3, w2)
    return out.reshape(B, Sq, D)
```

```python
import jax
import jax.numpy as jnp
from jax import lax
import jax.experimental.pallas as pl
import jax.experimental.pallas.tpu as pltpu

F32 = jnp.float32
BF16 = jnp.bfloat16

HQ = 32
DH = 192
LANE = 128
RA = 32
NJ = RA // 8
AH = DH // RA
HG = 5
HE = 4
NA = HG * AH
GROWS = HG * DH
JROT = 1
LEAD = 16

W2S = 4
TAIL_ROWS = 32
TAIL_GRAN = (5, 3, 2, 1, 1)

X_SEM, Q_SEM, F1_SEM, F2_SEM, O_SEM, K_SEM, V_SEM = 0, 1, 2, 3, 4, 5, 7
T_SEM = 0
N_SEM = V_SEM + 2 * NJ


def _kernel(x_hbm, k_hbm, v_hbm, wq_hbm, wo_hbm, w1_hbm, w3_hbm, w2_hbm,
            out_ref,
            x_v, wq_v, wo_v, w1_v, w3_v, w2_v, kbuf, vbuf, q_s, qblk, p_s, acc, hb_s,
            sems, *, B, D, S, W, F):
    NC = W // LANE
    NH = B * HQ
    NG = (NH - 2 * HE) // HG + 2
    S0 = S - W
    FS = F // W2S
    ALL = slice(None)

    def head0(g):
        if isinstance(g, int):
            return 0 if g == 0 else HE + HG * (g - 1)
        return HG * g - (HG - HE)

    def nheads(g):
        return HE if isinstance(g, int) and g in (0, NG - 1) else HG

    def rows8(j):
        return pl.ds(j * 8, 8) if isinstance(j, int) else pl.ds(pl.multiple_of(j * 8, 8), 8)

    def lanes(c, m=1, off=0):
        n = m * LANE
        if isinstance(c, int):
            return pl.ds(off + c * n, n)
        return pl.ds(pl.multiple_of(off + c * n, LANE), n)

    def k_copy(g, nh, j, c):
        slot = g % 2
        return pltpu.make_async_copy(
            k_hbm.at[pl.ds(head0(g) * AH, nh * AH), rows8(j), lanes(c, 1, S0)],
            kbuf.at[slot, pl.ds(0, nh * AH), rows8(j), lanes(c)],
            sems.at[K_SEM + slot])

    def v_copy(g, nh, j, c):
        slot = (g % 2) * NJ + j
        return pltpu.make_async_copy(
            v_hbm.at[pl.ds(head0(g) * AH, nh * AH), j, :, lanes(c, 1, S0)],
            vbuf.at[slot, pl.ds(0, nh * AH), :, lanes(c)],
            sems.at[V_SEM + slot])

    def wait_all(buf, sem):
        pltpu.make_async_copy(buf, buf, sems.at[sem]).wait()

    def w_copy(src, dst, idx, sem):
        return pltpu.make_async_copy(src.at[idx], dst.at[idx], sems.at[sem])

    def loop(lo, hi, fn):
        def body(i, carry):
            fn(i)
            return carry
        lax.fori_loop(lo, hi, body, 0)

    def issue_w13(j):
        for c in range(F // (4 * LANE)):
            w_copy(w1_hbm, w1_v, (ALL, rows8(j), lanes(c, 4)), F1_SEM).start(priority=0)
            w_copy(w3_hbm, w3_v, (ALL, rows8(j), lanes(c, 4)), F1_SEM).start(priority=1)

    def issue_w2(j):
        main = pl.ds(0, W2S - 1)
        w_copy(w2_hbm, w2_v, (main, rows8(j), ALL), F2_SEM).start(priority=0)
        w_copy(w2_hbm, w2_v, (main, rows8(j + FS // 16), ALL), F2_SEM).start(priority=1)

    def issue_wo(j):
        w_copy(wo_hbm, wo_v, (pl.ds(0, 4), j), O_SEM).start(priority=0)
        w_copy(wo_hbm, wo_v, (pl.ds(4, 4), j), O_SEM).start(priority=1)

    def issue_k_alone(g, j):
        def f(c):
            k_copy(g, nheads(g), j, c).start(priority=0)
            k_copy(g, nheads(g), j, c + NC // 2).start(priority=1)
        loop(0, NC // 2, f)

    def issue_pair(g, j, nk, nv):
        def f(c):
            k_copy(g + 1, nk, (j + JROT) % NJ, c).start(priority=0)
            v_copy(g, nv, j, c).start(priority=1)
        loop(0, NC, f)

    n_tail = sum(TAIL_GRAN)
    tail_sem = [T_SEM + t for t, n in enumerate(TAIL_GRAN) for _ in range(n)]
    t0_list = [(j, c) for j in range(NJ) for c in range(NC)
               if c < NC // 2 or (j == 0 and c < NC // 2 + n_tail // 2)]
    t1_list = [(j, c) for j in range(NJ) for c in range(NC) if (j, c) not in t0_list]
    t1_list += [(None, i) for i in range(n_tail)]
    assert len(t0_list) == len(t1_list)

    def issue_last(part):
        n = len(t0_list)
        for i in range(part * n // NJ, (part + 1) * n // NJ):
            v_copy(NG - 1, HE, *t0_list[i]).start(priority=0)
            j, c = t1_list[i]
            if j is None:
                w_copy(w2_hbm, w2_v, (W2S - 1, pl.ds(c * TAIL_ROWS, TAIL_ROWS), ALL),
                       tail_sem[c]).start(priority=1)
            else:
                v_copy(NG - 1, HE, j, c).start(priority=1)

    def qproj(xn, lo, hi):
        w = wq_v[:, :, lo:hi].reshape(D, hi - lo)
        q = jnp.dot(xn, w, preferred_element_type=F32)
        q_s[:, lo:hi] = q.astype(BF16).astype(F32)

    def build_qblk(g):
        row = lax.broadcasted_iota(jnp.int32, (8, GROWS), 0)
        col = lax.broadcasted_iota(jnp.int32, (8, GROWS), 1)
        diag = (col >= row * DH) & (col < (row + 1) * DH)
        h0, nh = head0(g), nheads(g)
        parts, h = [], h0
        while h < h0 + nh:
            b, hh = divmod(h, HQ)
            n = min(h0 + nh - h, HQ - hh)
            parts.append(q_s[b:b + 1, hh * DH:(hh + n) * DH])
            h += n
        if nh < HG:
            parts.append(jnp.zeros((1, (HG - nh) * DH), F32))
        flat = parts[0] if len(parts) == 1 else jnp.concatenate(parts, axis=1)
        qblk[g] = jnp.where(diag, jnp.broadcast_to(flat, (8, GROWS)), 0.0)

    def wait_k(g, nh):
        slot = g % 2
        wait_all(kbuf.at[slot, pl.ds(0, nh * AH)], K_SEM + slot)

    def scores_softmax(g, nh):
        kk = kbuf[g % 2, 0:nh * AH].reshape(nh * DH, W)
        qq = qblk[g][:, 0:nh * DH].astype(BF16)
        s = jnp.dot(qq, kk, preferred_element_type=F32) * (DH ** -0.5)
        m = jnp.max(s, axis=-1, keepdims=True)
        e = jnp.exp(s - m)
        l = jnp.sum(e, axis=-1, keepdims=True)
        p_s[...] = e * (1.0 / l)

    def pv_wo(g, j):
        nh = nheads(g)
        slot = (g % 2) * NJ + j
        wait_all(vbuf.at[slot, pl.ds(0, nh * AH)], V_SEM + slot)
        for hh in range(nh):
            h = head0(g) + hh
            b, hl = h // HQ, h % HQ
            pb = jnp.broadcast_to(p_s[hh:hh + 1, :], (8, W))
            tot = None
            for a in range(AH):
                prod = vbuf[slot, hh * AH + a].astype(F32) * pb
                parts = [prod[:, c * LANE:(c + 1) * LANE] for c in range(NC)]
                while len(parts) > 1:
                    parts = [parts[i] + parts[i + 1] for i in range(0, len(parts), 2)]
                o = jnp.sum(parts[0], axis=-1, keepdims=True)
                wrow = wo_v[hl // 4, (hl % 4) * (DH // 8) + NJ * a + j].astype(F32)
                tot = o * wrow if tot is None else tot + o * wrow
            acc[b] = acc[b] + tot

    wq_descs = [(ALL, rows8(j), lanes(c, 2)) for j in range(10) for c in range(HQ * DH // (2 * LANE))]
    n0 = (len(wq_descs) - LEAD) // 2
    for i in range(LEAD):
        w_copy(wq_hbm, wq_v, wq_descs[n0 + i], Q_SEM).start(priority=1)
    xcp = pltpu.make_async_copy(x_hbm, x_v, sems.at[X_SEM])
    xcp.start()
    for i in range(n0):
        w_copy(wq_hbm, wq_v, wq_descs[i], Q_SEM).start(priority=0)
        w_copy(wq_hbm, wq_v, wq_descs[n0 + LEAD + i], Q_SEM).start(priority=1)
    xcp.wait()
    x = x_v[...].astype(F32)
    mu = jnp.mean(x, axis=-1, keepdims=True)
    xc = x - mu
    var = jnp.mean(xc * xc, axis=-1, keepdims=True)
    xn4 = xc / jnp.sqrt(var + 1e-5)
    xn = jnp.concatenate([xn4, jnp.zeros((8 - B, D), F32)], axis=0).astype(BF16)
    loop(0, 16, issue_w13)
    wait_all(wq_v, Q_SEM)
    qproj(xn, 0, HQ * DH // 2)
    loop(0, FS // 16, issue_w2)
    qproj(xn, HQ * DH // 2, HQ * DH)
    loop(0, 32, issue_wo)
    for g in range(NG):
        build_qblk(g)
    wait_all(w1_v, F1_SEM)
    wait_all(w3_v, F1_SEM)
    gate = jnp.dot(xn, w1_v[...].reshape(D, F), preferred_element_type=F32)
    up = jnp.dot(xn, w3_v[...].reshape(D, F), preferred_element_type=F32)
    hmid = (gate * jax.nn.sigmoid(gate) * up).astype(BF16)
    loop(32, 64, issue_wo)
    FM = F - FS
    wait_all(w2_v.at[pl.ds(0, W2S - 1)], F2_SEM)
    ffn = jnp.dot(hmid[:, 0:FM], w2_v[0:W2S - 1].reshape(FM, D), preferred_element_type=F32)
    base = x + ffn[0:B, :]
    row8 = lax.broadcasted_iota(jnp.int32, (8, D), 0)
    for b in range(B):
        acc[b] = jnp.where(row8 == 0, jnp.broadcast_to(base[b:b + 1, :], (8, D)), 0.0)
    eye = (lax.broadcasted_iota(jnp.int32, (LANE, LANE), 0)
           == lax.broadcasted_iota(jnp.int32, (LANE, LANE), 1))
    hf = hmid.astype(F32)
    for b in range(B):
        for t in range(FS // LANE):
            hrow = hf[b:b + 1, FM + t * LANE:FM + (t + 1) * LANE]
            col = jnp.sum(jnp.where(eye, jnp.broadcast_to(hrow, (LANE, LANE)), 0.0),
                          axis=-1, keepdims=True)
            hb_s[b, t * LANE:(t + 1) * LANE, :] = jnp.broadcast_to(col, (LANE, LANE))
    loop(64, 96, issue_wo)
    for j in range(NJ):
        issue_k_alone(0, j)
    for j in range(NJ):
        issue_pair(0, j, HG, HE)
        if j == 2:
            wait_k(0, HE)
            scores_softmax(0, HE)
    wait_all(wo_v, O_SEM)
    for j in range(NJ):
        issue_pair(1, j, HG, HG)
        pv_wo(0, j)
    wait_k(1, HG)
    scores_softmax(1, HG)

    def group_body(g, carry):
        for j in range(NJ):
            pl.when(g < NG - 3)(lambda: issue_pair(g + 1, j, HG, HG))
            pl.when(g == NG - 3)(lambda: issue_pair(NG - 2, j, HE, HG))
            pl.when(g == NG - 2)(lambda: issue_last(j))
            pv_wo(g, j)
        pl.when(g < NG - 2)(lambda: wait_k(g + 1, HG))
        pl.when(g == NG - 2)(lambda: wait_k(NG - 1, HE))
        scores_softmax(g + 1, HG)
        return carry

    lax.fori_loop(1, NG - 1, group_body, 0)

    for j in range(NJ):
        pv_wo(NG - 1, j)
    tot = [acc[b] for b in range(B)]
    r0 = 0
    for t, n in enumerate(TAIL_GRAN):
        wait_all(w2_v.at[W2S - 1, pl.ds(r0, n * TAIL_ROWS)], T_SEM + t)
        for r in range(r0, r0 + n * TAIL_ROWS, 8):
            wrow = w2_v[W2S - 1, r:r + 8, :].astype(F32)
            for b in range(B):
                hb = hb_s[b, r:r + 8, :]
                tot[b] = tot[b] + jnp.concatenate([hb] * (D // LANE), axis=1) * wrow
        r0 += n * TAIL_ROWS
    res = jnp.concatenate([jnp.sum(t, axis=0, keepdims=True) for t in tot], axis=0)
    out_ref[...] = res.astype(out_ref.dtype)


@jax.jit
def pallas_parallel_sum__sliding_block_cached__glu_gated_swiglu__decode_kernel(
    A_x: jax.Array,
    A_k_cache: jax.Array,
    A_v_cache: jax.Array,
    A_wq: jax.Array,
    A_wo: jax.Array,
    B_x: jax.Array,
    B_w1: jax.Array,
    B_w3: jax.Array,
    B_w2: jax.Array,
):
    B, Sq, D = A_x.shape
    _, Hkv, S, Dh = A_k_cache.shape
    F = B_w1.shape[1]
    assert (B, Sq, D, Hkv, Dh, F) == (4, 1, 640, HQ, DH, 1536)
    W = min(4096, max(256, S // 4))
    assert W == 2048 and sum(TAIL_GRAN) * TAIL_ROWS == F // W2S

    kt = jnp.swapaxes(A_k_cache, 2, 3).reshape(B * HQ * AH, RA, S)
    vt = jnp.swapaxes(A_v_cache, 2, 3).reshape(B * HQ * AH, NJ, 8, S)
    x2 = A_x.reshape(B, D)
    wq = A_wq.reshape(8, D // 8, HQ * DH)
    wo = A_wo.reshape(8, HQ * DH // 64, 8, D)
    w1 = B_w1.reshape(5, D // 5, F)
    w3 = B_w3.reshape(5, D // 5, F)
    w2 = B_w2.reshape(W2S, F // W2S, D)
    NG = (B * HQ - 2 * HE) // HG + 2

    kern = lambda *refs: _kernel(*refs, B=B, D=D, S=S, W=W, F=F)
    out = pl.pallas_call(
        kern,
        in_specs=[pl.BlockSpec(memory_space=pl.ANY)] * 8,
        out_specs=pl.BlockSpec(memory_space=pltpu.VMEM),
        out_shape=jax.ShapeDtypeStruct((B, D), A_x.dtype),
        scratch_shapes=[
            pltpu.VMEM((B, D), BF16),
            pltpu.VMEM(wq.shape, BF16),
            pltpu.VMEM(wo.shape, BF16),
            pltpu.VMEM(w1.shape, BF16),
            pltpu.VMEM(w3.shape, BF16),
            pltpu.VMEM(w2.shape, BF16),
            pltpu.VMEM((2, NA, RA, W), BF16),
            pltpu.VMEM((2 * NJ, NA, 8, W), BF16),
            pltpu.VMEM((8, HQ * DH), F32),
            pltpu.VMEM((NG, 8, GROWS), F32),
            pltpu.VMEM((8, W), F32),
            pltpu.VMEM((B, 8, D), F32),
            pltpu.VMEM((B, F // W2S, LANE), F32),
            pltpu.SemaphoreType.DMA((N_SEM,)),
        ],
        compiler_params=pltpu.CompilerParams(vmem_limit_bytes=100 * 1024 * 1024,
                                             disable_semaphore_checks=True),
    )(x2, kt, vt, wq, wo, w1, w3, w2)
    return out.reshape(B, Sq, D)
```

```python
import jax
import jax.numpy as jnp
from jax import lax
import jax.experimental.pallas as pl
import jax.experimental.pallas.tpu as pltpu

F32 = jnp.float32
BF16 = jnp.bfloat16

HQ = 32
DH = 192
LANE = 128
RA = 32
NJ = RA // 8
AH = DH // RA
HG = 5
HE = 4
NA = HG * AH
GROWS = HG * DH
JROT = 1
LEAD = 16

W2S = 4
TAIL_ROWS = 32
TAIL_GRAN = (5, 3, 2, 1, 1)

X_SEM, Q_SEM, F1_SEM, F2_SEM, O_SEM, K_SEM, V_SEM = 0, 1, 2, 3, 4, 5, 7
T_SEM = 0
N_SEM = V_SEM + 2 * NJ


def _kernel(x_hbm, k_hbm, v_hbm, wq_hbm, wo_hbm, w1_hbm, w3_hbm, w2_hbm,
            out_ref,
            x_v, wq_v, wo_v, w1_v, w3_v, w2_v, kbuf, vbuf, q_s, qblk, p_s, acc, hb_s,
            sems, *, B, D, S, W, F):
    NC = W // LANE
    NH = B * HQ
    NG = (NH - 2 * HE) // HG + 2
    S0 = S - W
    FS = F // W2S
    ALL = slice(None)

    def head0(g):
        if isinstance(g, int):
            return 0 if g == 0 else HE + HG * (g - 1)
        return HG * g - (HG - HE)

    def nheads(g):
        return HE if isinstance(g, int) and g in (0, NG - 1) else HG

    def rows8(j):
        return pl.ds(j * 8, 8) if isinstance(j, int) else pl.ds(pl.multiple_of(j * 8, 8), 8)

    def lanes(c, m=1, off=0):
        n = m * LANE
        if isinstance(c, int):
            return pl.ds(off + c * n, n)
        return pl.ds(pl.multiple_of(off + c * n, LANE), n)

    def k_copy(g, nh, j, c):
        slot = g % 2
        return pltpu.make_async_copy(
            k_hbm.at[pl.ds(head0(g) * AH, nh * AH), rows8(j), lanes(c, 1, S0)],
            kbuf.at[slot, pl.ds(0, nh * AH), rows8(j), lanes(c)],
            sems.at[K_SEM + slot])

    def v_copy(g, nh, j, c):
        slot = (g % 2) * NJ + j
        return pltpu.make_async_copy(
            v_hbm.at[pl.ds(head0(g) * AH, nh * AH), j, :, lanes(c, 1, S0)],
            vbuf.at[slot, pl.ds(0, nh * AH), :, lanes(c)],
            sems.at[V_SEM + slot])

    def wait_all(buf, sem):
        pltpu.make_async_copy(buf, buf, sems.at[sem]).wait()

    def w_copy(src, dst, idx, sem):
        return pltpu.make_async_copy(src.at[idx], dst.at[idx], sems.at[sem])

    def loop(lo, hi, fn):
        def body(i, carry):
            fn(i)
            return carry
        lax.fori_loop(lo, hi, body, 0)

    def issue_w13(j):
        for c in range(F // (4 * LANE)):
            w_copy(w1_hbm, w1_v, (ALL, rows8(j), lanes(c, 4)), F1_SEM).start(priority=0)
            w_copy(w3_hbm, w3_v, (ALL, rows8(j), lanes(c, 4)), F1_SEM).start(priority=1)

    def issue_w2(j):
        main = pl.ds(0, W2S - 1)
        w_copy(w2_hbm, w2_v, (main, rows8(j), ALL), F2_SEM).start(priority=0)
        w_copy(w2_hbm, w2_v, (main, rows8(j + FS // 16), ALL), F2_SEM).start(priority=1)

    def issue_wo(j):
        w_copy(wo_hbm, wo_v, (pl.ds(0, 4), j), O_SEM).start(priority=0)
        w_copy(wo_hbm, wo_v, (pl.ds(4, 4), j), O_SEM).start(priority=1)

    def issue_k_alone(g, j):
        def f(c):
            k_copy(g, nheads(g), j, c).start(priority=0)
            k_copy(g, nheads(g), j, c + NC // 2).start(priority=1)
        loop(0, NC // 2, f)

    def issue_pair(g, j, nk, nv):
        def f(c):
            k_copy(g + 1, nk, (j + JROT) % NJ, c).start(priority=0)
            v_copy(g, nv, j, c).start(priority=1)
        loop(0, NC, f)

    n_tail = sum(TAIL_GRAN)
    tail_sem = [T_SEM + t for t, n in enumerate(TAIL_GRAN) for _ in range(n)]
    t0_list = [(j, c) for j in range(NJ) for c in range(NC)
               if c < NC // 2 or (j == 0 and c < NC // 2 + n_tail // 2)]
    t1_list = [(j, c) for j in range(NJ) for c in range(NC) if (j, c) not in t0_list]
    t1_list += [(None, i) for i in range(n_tail)]
    assert len(t0_list) == len(t1_list)

    def issue_last(part):
        n = len(t0_list)
        for i in range(part * n // NJ, (part + 1) * n // NJ):
            v_copy(NG - 1, HE, *t0_list[i]).start(priority=0)
            j, c = t1_list[i]
            if j is None:
                w_copy(w2_hbm, w2_v, (W2S - 1, pl.ds(c * TAIL_ROWS, TAIL_ROWS), ALL),
                       tail_sem[c]).start(priority=1)
            else:
                v_copy(NG - 1, HE, j, c).start(priority=1)

    def qproj(xn, lo, hi):
        w = wq_v[:, :, lo:hi].reshape(D, hi - lo)
        q = jnp.dot(xn, w, preferred_element_type=F32)
        q_s[:, lo:hi] = q.astype(BF16).astype(F32)

    def build_qblk(g):
        row = lax.broadcasted_iota(jnp.int32, (8, GROWS), 0)
        col = lax.broadcasted_iota(jnp.int32, (8, GROWS), 1)
        diag = (col >= row * DH) & (col < (row + 1) * DH)
        h0, nh = head0(g), nheads(g)
        parts, h = [], h0
        while h < h0 + nh:
            b, hh = divmod(h, HQ)
            n = min(h0 + nh - h, HQ - hh)
            parts.append(q_s[b:b + 1, hh * DH:(hh + n) * DH])
            h += n
        if nh < HG:
            parts.append(jnp.zeros((1, (HG - nh) * DH), F32))
        flat = parts[0] if len(parts) == 1 else jnp.concatenate(parts, axis=1)
        qblk[g] = jnp.where(diag, jnp.broadcast_to(flat, (8, GROWS)), 0.0)

    def wait_k(g, nh):
        slot = g % 2
        wait_all(kbuf.at[slot, pl.ds(0, nh * AH)], K_SEM + slot)

    def scores_softmax(g, nh):
        kk = kbuf[g % 2, 0:nh * AH].reshape(nh * DH, W)
        qq = qblk[g][:, 0:nh * DH].astype(BF16)
        s = jnp.dot(qq, kk, preferred_element_type=F32) * (DH ** -0.5)
        m = jnp.max(s, axis=-1, keepdims=True)
        e = jnp.exp(s - m)
        l = jnp.sum(e, axis=-1, keepdims=True)
        p_s[g % 2] = e * (1.0 / l)

    def pv_wo(g, j):
        nh = nheads(g)
        slot = (g % 2) * NJ + j
        wait_all(vbuf.at[slot, pl.ds(0, nh * AH)], V_SEM + slot)
        for hh in range(nh):
            h = head0(g) + hh
            b, hl = h // HQ, h % HQ
            pb = jnp.broadcast_to(p_s[g % 2, hh:hh + 1, :], (8, W))
            tot = None
            for a in range(AH):
                prod = vbuf[slot, hh * AH + a].astype(F32) * pb
                parts = [prod[:, c * LANE:(c + 1) * LANE] for c in range(NC)]
                while len(parts) > 1:
                    parts = [parts[i] + parts[i + 1] for i in range(0, len(parts), 2)]
                o = jnp.sum(parts[0], axis=-1, keepdims=True)
                wrow = wo_v[hl // 4, (hl % 4) * (DH // 8) + NJ * a + j].astype(F32)
                tot = o * wrow if tot is None else tot + o * wrow
            acc[b] = acc[b] + tot

    wq_descs = [(ALL, rows8(j), lanes(c, 2)) for j in range(10) for c in range(HQ * DH // (2 * LANE))]
    n0 = (len(wq_descs) - LEAD) // 2
    for i in range(LEAD):
        w_copy(wq_hbm, wq_v, wq_descs[n0 + i], Q_SEM).start(priority=1)
    xcp = pltpu.make_async_copy(x_hbm, x_v, sems.at[X_SEM])
    xcp.start()
    for i in range(n0):
        w_copy(wq_hbm, wq_v, wq_descs[i], Q_SEM).start(priority=0)
        w_copy(wq_hbm, wq_v, wq_descs[n0 + LEAD + i], Q_SEM).start(priority=1)
    xcp.wait()
    x = x_v[...].astype(F32)
    mu = jnp.mean(x, axis=-1, keepdims=True)
    xc = x - mu
    var = jnp.mean(xc * xc, axis=-1, keepdims=True)
    xn4 = xc / jnp.sqrt(var + 1e-5)
    xn = jnp.concatenate([xn4, jnp.zeros((8 - B, D), F32)], axis=0).astype(BF16)
    loop(0, 16, issue_w13)
    wait_all(wq_v, Q_SEM)
    qproj(xn, 0, HQ * DH // 2)
    loop(0, FS // 16, issue_w2)
    qproj(xn, HQ * DH // 2, HQ * DH)
    loop(0, 32, issue_wo)
    for g in range(NG):
        build_qblk(g)
    wait_all(w1_v, F1_SEM)
    wait_all(w3_v, F1_SEM)
    gate = jnp.dot(xn, w1_v[...].reshape(D, F), preferred_element_type=F32)
    up = jnp.dot(xn, w3_v[...].reshape(D, F), preferred_element_type=F32)
    hmid = (gate * jax.nn.sigmoid(gate) * up).astype(BF16)
    loop(32, 64, issue_wo)
    FM = F - FS
    wait_all(w2_v.at[pl.ds(0, W2S - 1)], F2_SEM)
    ffn = jnp.dot(hmid[:, 0:FM], w2_v[0:W2S - 1].reshape(FM, D), preferred_element_type=F32)
    base = x + ffn[0:B, :]
    row8 = lax.broadcasted_iota(jnp.int32, (8, D), 0)
    for b in range(B):
        acc[b] = jnp.where(row8 == 0, jnp.broadcast_to(base[b:b + 1, :], (8, D)), 0.0)
    eye = (lax.broadcasted_iota(jnp.int32, (LANE, LANE), 0)
           == lax.broadcasted_iota(jnp.int32, (LANE, LANE), 1))
    hf = hmid.astype(F32)
    for b in range(B):
        for t in range(FS // LANE):
            hrow = hf[b:b + 1, FM + t * LANE:FM + (t + 1) * LANE]
            col = jnp.sum(jnp.where(eye, jnp.broadcast_to(hrow, (LANE, LANE)), 0.0),
                          axis=-1, keepdims=True)
            hb_s[b, t * LANE:(t + 1) * LANE, :] = jnp.broadcast_to(col, (LANE, LANE))
    loop(64, 96, issue_wo)
    for j in range(NJ):
        issue_k_alone(0, j)
    for j in range(NJ):
        issue_pair(0, j, HG, HE)
        if j == 2:
            wait_k(0, HE)
            scores_softmax(0, HE)
    wait_all(wo_v, O_SEM)
    for j in range(NJ):
        issue_pair(1, j, HG, HG)
        pv_wo(0, j)
    wait_k(1, HG)
    scores_softmax(1, HG)

    def group_body(g, carry):
        for j in range(NJ):
            pl.when(g < NG - 3)(lambda: issue_pair(g + 1, j, HG, HG))
            pl.when(g == NG - 3)(lambda: issue_pair(NG - 2, j, HE, HG))
            pl.when(g == NG - 2)(lambda: issue_last(j))
            if j == NJ - 1:
                pl.when(g < NG - 2)(lambda: wait_k(g + 1, HG))
                pl.when(g == NG - 2)(lambda: wait_k(NG - 1, HE))
                scores_softmax(g + 1, HG)
            pv_wo(g, j)
        return carry

    lax.fori_loop(1, NG - 1, group_body, 0)

    for j in range(NJ):
        pv_wo(NG - 1, j)
    tot = [acc[b] for b in range(B)]
    r0 = 0
    for t, n in enumerate(TAIL_GRAN):
        wait_all(w2_v.at[W2S - 1, pl.ds(r0, n * TAIL_ROWS)], T_SEM + t)
        for r in range(r0, r0 + n * TAIL_ROWS, 8):
            wrow = w2_v[W2S - 1, r:r + 8, :].astype(F32)
            for b in range(B):
                hb = hb_s[b, r:r + 8, :]
                tot[b] = tot[b] + jnp.concatenate([hb] * (D // LANE), axis=1) * wrow
        r0 += n * TAIL_ROWS
    res = jnp.concatenate([jnp.sum(t, axis=0, keepdims=True) for t in tot], axis=0)
    out_ref[...] = res.astype(out_ref.dtype)


@jax.jit
def pallas_parallel_sum__sliding_block_cached__glu_gated_swiglu__decode_kernel(
    A_x: jax.Array,
    A_k_cache: jax.Array,
    A_v_cache: jax.Array,
    A_wq: jax.Array,
    A_wo: jax.Array,
    B_x: jax.Array,
    B_w1: jax.Array,
    B_w3: jax.Array,
    B_w2: jax.Array,
):
    B, Sq, D = A_x.shape
    _, Hkv, S, Dh = A_k_cache.shape
    F = B_w1.shape[1]
    assert (B, Sq, D, Hkv, Dh, F) == (4, 1, 640, HQ, DH, 1536)
    W = min(4096, max(256, S // 4))
    assert W == 2048 and sum(TAIL_GRAN) * TAIL_ROWS == F // W2S

    kt = jnp.swapaxes(A_k_cache, 2, 3).reshape(B * HQ * AH, RA, S)
    vt = jnp.swapaxes(A_v_cache, 2, 3).reshape(B * HQ * AH, NJ, 8, S)
    x2 = A_x.reshape(B, D)
    wq = A_wq.reshape(8, D // 8, HQ * DH)
    wo = A_wo.reshape(8, HQ * DH // 64, 8, D)
    w1 = B_w1.reshape(5, D // 5, F)
    w3 = B_w3.reshape(5, D // 5, F)
    w2 = B_w2.reshape(W2S, F // W2S, D)
    NG = (B * HQ - 2 * HE) // HG + 2

    kern = lambda *refs: _kernel(*refs, B=B, D=D, S=S, W=W, F=F)
    out = pl.pallas_call(
        kern,
        in_specs=[pl.BlockSpec(memory_space=pl.ANY)] * 8,
        out_specs=pl.BlockSpec(memory_space=pltpu.VMEM),
        out_shape=jax.ShapeDtypeStruct((B, D), A_x.dtype),
        scratch_shapes=[
            pltpu.VMEM((B, D), BF16),
            pltpu.VMEM(wq.shape, BF16),
            pltpu.VMEM(wo.shape, BF16),
            pltpu.VMEM(w1.shape, BF16),
            pltpu.VMEM(w3.shape, BF16),
            pltpu.VMEM(w2.shape, BF16),
            pltpu.VMEM((2, NA, RA, W), BF16),
            pltpu.VMEM((2 * NJ, NA, 8, W), BF16),
            pltpu.VMEM((8, HQ * DH), F32),
            pltpu.VMEM((NG, 8, GROWS), F32),
            pltpu.VMEM((2, 8, W), F32),
            pltpu.VMEM((B, 8, D), F32),
            pltpu.VMEM((B, F // W2S, LANE), F32),
            pltpu.SemaphoreType.DMA((N_SEM,)),
        ],
        compiler_params=pltpu.CompilerParams(vmem_limit_bytes=100 * 1024 * 1024,
                                             disable_semaphore_checks=True),
    )(x2, kt, vt, wq, wo, w1, w3, w2)
    return out.reshape(B, Sq, D)
```

```python
import jax
import jax.numpy as jnp
from jax import lax
import jax.experimental.pallas as pl
import jax.experimental.pallas.tpu as pltpu

F32 = jnp.float32
BF16 = jnp.bfloat16
ALL = slice(None)

HQ = 32
DH = 192
LANE = 128
RA = 32
NJ = RA // 8
HG = 5
HE = 4
GROWS = HG * DH
LEAD = 16
UNROLL = 4

MODE = "D2"
LA = 4
ORDER = (("v", 0), ("v", 1), ("k", 0), ("v", 2), ("v", 3), ("k", 2))
if MODE == "A":
    NE, NR = 2, 3
    UNITS = [(16, (1 + 2 * (u // 3), ALL, u % 3, 0), ORDER[u] + (ALL, ALL, 0)) for u in range(6)]
    FIRST = [(16, (3, ALL, u, 0), ("k", u, ALL, ALL, 0)) for u in range(3)]
    SMALL = [(ALL, r) for r in range(3)]
    LAST_COLS = (5, 5, 5, 5)
elif MODE == "D1":
    NE, NR = 2, 3
    UNITS = [(16, (1, u // 3, u % 3, 0), ORDER[u] + (ALL, ALL, 0)) for u in range(6)]
    UNITS.append((8, (3, ALL, ALL, 0), ("k", 3, ALL, ALL, 8)))
    FIRST = [(16, (3, ALL, u, 0), ("k", u, ALL, ALL, 0)) for u in range(3)]
    SMALL = [(ALL, r) for r in range(3)]
    LAST_COLS = (5, 5, 5, 5)
else:
    NE, NR = 3, 2
    UNITS = [(16, (1, u // 2, u % 2, 0), ORDER[u] + (ALL, ALL, 0)) for u in range(6)]
    UNITS.append((16, (3, ALL, 0, 0), ("k", 3, ALL, 1, 0)))
    FIRST = [(16, (3, u // 2, u % 2, 0), ("k", u // 2, ALL, u % 2, 0)) for u in range(6)]
    SMALL = [(e, r) for e in range(3) for r in range(2)]
    LAST_COLS = (3, 3, 2, 2)
NU = len(UNITS)

W2S = 4
W2_MAIN = 24
W2_SMALL = 3
TAIL_GRAN = (3, 3, 2, 2, 1, 1)
LAST_ISSUE = (16, 16, 16, 16, 24, 24)

X_SEM, Q_SEM, F1_SEM, F2_SEM, O_SEM, K_SEM, V_SEM = 0, 1, 2, 3, 4, 5, 7
T_SEM = V_SEM + 2 * NJ
N_SEM = T_SEM + len(TAIL_GRAN)


def _kernel(x_hbm, k_hbm, v_hbm, wq_hbm, wo_hbm, w1_hbm, w3_hbm, w2_hbm,
            out_ref,
            x_v, wq_v, wo_v, w1_v, w3_v, w2_v, kbuf, vbuf, q_s, qblk, p_s, acc, h_s, hb_s,
            sems, *, B, D, S, W, F):
    NC = W // LANE
    NG = (B * HQ - 2 * HE) // HG + 2
    S0 = S - W
    FS = F // W2S

    def head0(g):
        if isinstance(g, int):
            return 0 if g == 0 else HE + HG * (g - 1)
        return HG * g - (HG - HE)

    def nheads(g):
        return HE if isinstance(g, int) and g in (0, NG - 1) else HG

    def rows8(j):
        return pl.ds(j * 8, 8) if isinstance(j, int) else pl.ds(pl.multiple_of(j * 8, 8), 8)

    def lanes(c, m=1, off=0):
        n = m * LANE
        if isinstance(c, int):
            return pl.ds(off + c * n, n)
        return pl.ds(pl.multiple_of(off + c * n, LANE), n)

    def k_copy(g, nh, j, e, r, c):
        slot = g % 2
        return pltpu.make_async_copy(
            k_hbm.at[pl.ds(head0(g), nh), e, r, rows8(j), lanes(c, 1, S0)],
            kbuf.at[slot, pl.ds(0, nh), e, r, rows8(j), lanes(c)],
            sems.at[K_SEM + slot])

    def v_copy(g, nh, j, e, r, c):
        slot = (g % 2) * NJ + j
        return pltpu.make_async_copy(
            v_hbm.at[pl.ds(head0(g), nh), e, r, j, :, lanes(c, 1, S0)],
            vbuf.at[slot, pl.ds(0, nh), e, r, :, lanes(c)],
            sems.at[V_SEM + slot])

    def wait_all(buf, sem):
        pltpu.make_async_copy(buf, buf, sems.at[sem]).wait()

    def w_copy(src, dst, idx, sem):
        return pltpu.make_async_copy(src.at[idx], dst.at[idx], sems.at[sem])

    def loop(lo, hi, fn, unroll=1):
        def body(i, carry):
            fn(i)
            return carry
        lax.fori_loop(lo, hi, body, 0, unroll=unroll)

    def issue_w13(j):
        for c in range(F // (4 * LANE)):
            w_copy(w1_hbm, w1_v, (ALL, rows8(j), lanes(c, 4)), F1_SEM).start(priority=0)
            w_copy(w3_hbm, w3_v, (ALL, rows8(j), lanes(c, 4)), F1_SEM).start(priority=1)

    def issue_w2(j):
        w_copy(w2_hbm, w2_v, (ALL, rows8(j), ALL), F2_SEM).start(priority=0)
        w_copy(w2_hbm, w2_v, (ALL, rows8(j + W2_MAIN // 2), ALL), F2_SEM).start(priority=1)

    def issue_wo(j):
        w_copy(wo_hbm, wo_v, (pl.ds(0, 4), j), O_SEM).start(priority=0)
        w_copy(wo_hbm, wo_v, (pl.ds(4, 4), j), O_SEM).start(priority=1)

    def issue_unit(g, unit, nk, nv):
        n, (j0, e0, r0, c0), (which, j1, e1, r1, c1) = unit

        def f(c):
            k_copy(g + 1, nk, j0, e0, r0, c + c0).start(priority=0)
            if which == "k":
                k_copy(g + 1, nk, j1, e1, r1, c + c1).start(priority=1)
            else:
                v_copy(g, nv, j1, e1, r1, c + c1).start(priority=1)
        loop(0, n, f, UNROLL)

    W2_TAIL = FS // 8 - sum(TAIL_GRAN)
    tail_sem = {j: F2_SEM for j in range(W2_MAIN, W2_TAIL)}
    for t, n in enumerate(TAIL_GRAN):
        for _ in range(n):
            tail_sem[W2_MAIN + len(tail_sem)] = T_SEM + t
    t0_list, t1_list = [], []
    for j, c0 in enumerate(LAST_COLS):
        t0_list += [(j, e, r, c) for e, r in SMALL for c in range(c0)]
        t1_list += [(j, ALL, ALL, c) for c in range(c0, NC)]
    t0_list += [(a, j) for j in range(W2_MAIN, W2_MAIN + W2_SMALL) for a in range(W2S)]
    t1_list += [(ALL, j) for j in range(W2_MAIN + W2_SMALL, FS // 8)]
    n_last = max(len(t0_list), len(t1_list))

    def issue_last(lo, hi):
        for i in range(lo, min(hi, n_last)):
            for prio, lst in enumerate((t0_list, t1_list)):
                if i >= len(lst):
                    continue
                d = lst[i]
                if len(d) == 2:
                    cp = w_copy(w2_hbm, w2_v, (d[0], rows8(d[1]), ALL), tail_sem[d[1]])
                else:
                    cp = v_copy(NG - 1, HE, *d)
                cp.start(priority=prio)

    def qproj(xn, lo, hi):
        w = wq_v[:, :, lo:hi].reshape(D, hi - lo)
        q = jnp.dot(xn, w, preferred_element_type=F32)
        q_s[:, lo:hi] = q.astype(BF16).astype(F32)

    def build_qblk(g):
        h0, nh = head0(g), nheads(g)
        row = lax.broadcasted_iota(jnp.int32, (8, nh * DH), 0)
        col = lax.broadcasted_iota(jnp.int32, (8, nh * DH), 1)
        diag = (col >= row * DH) & (col < (row + 1) * DH)
        parts, h = [], h0
        while h < h0 + nh:
            b, hh = divmod(h, HQ)
            n = min(h0 + nh - h, HQ - hh)
            parts.append(q_s[b:b + 1, hh * DH:(hh + n) * DH])
            h += n
        flat = parts[0] if len(parts) == 1 else jnp.concatenate(parts, axis=1)
        qblk[g, :, 0:nh * DH] = jnp.where(diag, jnp.broadcast_to(flat, (8, nh * DH)), 0.0)

    def scores_softmax(g):
        nh = nheads(g)
        slot = g % 2
        wait_all(kbuf.at[slot, pl.ds(0, nh)], K_SEM + slot)
        kk = kbuf[slot, 0:nh].reshape(nh * DH, W)
        qq = qblk[g, :, 0:nh * DH].astype(BF16)
        s = jnp.dot(qq, kk, preferred_element_type=F32) * (DH ** -0.5)
        m = jnp.max(s, axis=-1, keepdims=True)
        e = jnp.exp(s - m)
        l = jnp.sum(e, axis=-1, keepdims=True)
        p_s[slot] = e * (1.0 / l)

    def pv_wo(g, j):
        nh = nheads(g)
        slot = (g % 2) * NJ + j
        wait_all(vbuf.at[slot, pl.ds(0, nh)], V_SEM + slot)
        for hh in range(nh):
            h = head0(g) + hh
            b, hl = h // HQ, h % HQ
            pb = jnp.broadcast_to(p_s[g % 2, hh:hh + 1, :], (8, W))
            tot = None
            for a in range(NE * NR):
                prod = vbuf[slot, hh, a // NR, a % NR].astype(F32) * pb
                parts = [prod[:, c * LANE:(c + 1) * LANE] for c in range(NC)]
                while len(parts) > 1:
                    parts = [parts[i] + parts[i + 1] for i in range(0, len(parts), 2)]
                o = jnp.sum(parts[0], axis=-1, keepdims=True)
                wrow = wo_v[hl // 4, (hl % 4) * (DH // 8) + NJ * a + j].astype(F32)
                tot = o * wrow if tot is None else tot + o * wrow
            acc[b] = acc[b] + tot

    def consume(g, u):
        if u == NU - 1:
            scores_softmax(g + 1)
        elif UNITS[u][2][0] == "v":
            pv_wo(g, UNITS[u][2][1])

    def ffn_down(lo, hi):
        lo, hi = lo * 8, hi * 8
        wait_all(w2_v.at[:, pl.ds(lo, hi - lo)], F2_SEM)
        out = None
        for a in range(W2S):
            part = jnp.dot(h_s[:, a * FS + lo:a * FS + hi].astype(BF16), w2_v[a, lo:hi, :],
                           preferred_element_type=F32)
            out = part if out is None else out + part
        return out

    def in_row0(v, b):
        row8 = lax.broadcasted_iota(jnp.int32, (8, D), 0)
        return jnp.where(row8 == 0, jnp.broadcast_to(v[b:b + 1, :], (8, D)), 0.0)

    wq_descs = [(ALL, rows8(j), lanes(c, 4))
                for j in range(16) for c in range(HQ * DH // (4 * LANE))]
    n0 = (len(wq_descs) - LEAD) // 2
    for i in range(LEAD):
        w_copy(wq_hbm, wq_v, wq_descs[n0 + i], Q_SEM).start(priority=1)
    xcp = pltpu.make_async_copy(x_hbm, x_v, sems.at[X_SEM])
    xcp.start()
    for i in range(n0):
        w_copy(wq_hbm, wq_v, wq_descs[i], Q_SEM).start(priority=0)
        w_copy(wq_hbm, wq_v, wq_descs[n0 + LEAD + i], Q_SEM).start(priority=1)
    xcp.wait()
    x = x_v[...].astype(F32)
    mu = jnp.mean(x, axis=-1, keepdims=True)
    xc = x - mu
    var = jnp.mean(xc * xc, axis=-1, keepdims=True)
    xn4 = xc / jnp.sqrt(var + 1e-5)
    xn = jnp.concatenate([xn4, jnp.zeros((8 - B, D), F32)], axis=0).astype(BF16)
    loop(0, 16, issue_w13)
    wait_all(wq_v, Q_SEM)
    qproj(xn, 0, HQ * DH // 2)
    loop(0, W2_MAIN // 2, issue_w2)
    qproj(xn, HQ * DH // 2, HQ * DH)
    loop(0, 32, issue_wo)
    for g in range(NG):
        build_qblk(g)
    wait_all(w1_v, F1_SEM)
    wait_all(w3_v, F1_SEM)
    gate = jnp.dot(xn, w1_v[...].reshape(D, F), preferred_element_type=F32)
    up = jnp.dot(xn, w3_v[...].reshape(D, F), preferred_element_type=F32)
    h_s[...] = (gate * jax.nn.sigmoid(gate) * up).astype(BF16).astype(F32)
    loop(32, 64, issue_wo)
    base = x + ffn_down(0, W2_MAIN)[0:B, :]
    for b in range(B):
        acc[b] = in_row0(base, b)
    eye = (lax.broadcasted_iota(jnp.int32, (LANE, LANE), 0)
           == lax.broadcasted_iota(jnp.int32, (LANE, LANE), 1))
    for b in range(B):
        for a in range(W2S):
            hrow = h_s[b:b + 1, (a + 1) * FS - LANE:(a + 1) * FS]
            col = jnp.sum(jnp.where(eye, jnp.broadcast_to(hrow, (LANE, LANE)), 0.0),
                          axis=-1, keepdims=True)
            hb_s[b, a] = jnp.broadcast_to(col, (LANE, LANE))
    loop(64, 96, issue_wo)
    for unit in FIRST:
        issue_unit(-1, unit, HE, None)

    def step(g, issue, first=False):
        for u in range(NU):
            issue(UNITS[u])
            if u >= LA:
                consume(g, u - LA)
            elif not first:
                consume(g - 1, u - LA + NU)
            elif u == LA - 1:
                wait_all(wo_v, O_SEM)
                scores_softmax(0)

    step(0, lambda unit: issue_unit(0, unit, HG, HE), first=True)
    step(1, lambda unit: issue_unit(1, unit, HG, HG))

    def group_body(g, carry):
        def issue(unit):
            pl.when(g < NG - 2)(lambda: issue_unit(g, unit, HG, HG))
            pl.when(g == NG - 2)(lambda: issue_unit(NG - 2, unit, HE, HG))
        step(g, issue)
        return carry

    lax.fori_loop(2, NG - 1, group_body, 0)

    todo = [lambda u=u: consume(NG - 2, u) for u in range(NU - LA, NU)]
    todo += [lambda j=j: pv_wo(NG - 1, j) for j in range(NJ)]
    pos = 0
    for i, fn in enumerate(todo):
        n = LAST_ISSUE[i] if i < len(LAST_ISSUE) else 0
        issue_last(pos, pos + n)
        pos += n
        fn()
    assert pos >= n_last
    tot = [acc[b] for b in range(B)]
    if W2_MAIN < W2_TAIL:
        mid = ffn_down(W2_MAIN, W2_TAIL)
        tot = [tot[b] + in_row0(mid, b) for b in range(B)]
    j0 = W2_TAIL
    for t, n in enumerate(TAIL_GRAN):
        wait_all(w2_v.at[:, pl.ds(j0 * 8, n * 8)], T_SEM + t)
        for j in range(j0, j0 + n):
            for a in range(W2S):
                wrow = w2_v[a, j * 8:j * 8 + 8, :].astype(F32)
                r = j * 8 - (FS - LANE)
                for b in range(B):
                    hb = hb_s[b, a, r:r + 8, :]
                    tot[b] = tot[b] + jnp.concatenate([hb] * (D // LANE), axis=1) * wrow
        j0 += n
    res = jnp.concatenate([jnp.sum(t, axis=0, keepdims=True) for t in tot], axis=0)
    out_ref[...] = res.astype(out_ref.dtype)


@jax.jit
def pallas_parallel_sum__sliding_block_cached__glu_gated_swiglu__decode_kernel(
    A_x: jax.Array,
    A_k_cache: jax.Array,
    A_v_cache: jax.Array,
    A_wq: jax.Array,
    A_wo: jax.Array,
    B_x: jax.Array,
    B_w1: jax.Array,
    B_w3: jax.Array,
    B_w2: jax.Array,
):
    B, Sq, D = A_x.shape
    _, Hkv, S, Dh = A_k_cache.shape
    F = B_w1.shape[1]
    assert (B, Sq, D, Hkv, Dh, F) == (4, 1, 640, HQ, DH, 1536)
    W = min(4096, max(256, S // 4))
    assert W == 2048 and sum(TAIL_GRAN) * 8 <= LANE

    kt = jnp.swapaxes(A_k_cache, 2, 3).reshape(B * HQ, NE, NR, RA, S)
    vt = jnp.swapaxes(A_v_cache, 2, 3).reshape(B * HQ, NE, NR, NJ, 8, S)
    x2 = A_x.reshape(B, D)
    wq = A_wq.reshape(5, D // 5, HQ * DH)
    wo = A_wo.reshape(8, HQ * DH // 64, 8, D)
    w1 = B_w1.reshape(5, D // 5, F)
    w3 = B_w3.reshape(5, D // 5, F)
    w2 = B_w2.reshape(W2S, F // W2S, D)
    NG = (B * HQ - 2 * HE) // HG + 2

    kern = lambda *refs: _kernel(*refs, B=B, D=D, S=S, W=W, F=F)
    out = pl.pallas_call(
        kern,
        in_specs=[pl.BlockSpec(memory_space=pl.ANY)] * 8,
        out_specs=pl.BlockSpec(memory_space=pltpu.VMEM),
        out_shape=jax.ShapeDtypeStruct((B, D), A_x.dtype),
        scratch_shapes=[
            pltpu.VMEM((B, D), BF16),
            pltpu.VMEM(wq.shape, BF16),
            pltpu.VMEM(wo.shape, BF16),
            pltpu.VMEM(w1.shape, BF16),
            pltpu.VMEM(w3.shape, BF16),
            pltpu.VMEM(w2.shape, BF16),
            pltpu.VMEM((2, HG, NE, NR, RA, W), BF16),
            pltpu.VMEM((2 * NJ, HG, NE, NR, 8, W), BF16),
            pltpu.VMEM((8, HQ * DH), F32),
            pltpu.VMEM((NG, 8, GROWS), F32),
            pltpu.VMEM((2, 8, W), F32),
            pltpu.VMEM((B, 8, D), F32),
            pltpu.VMEM((8, F), F32),
            pltpu.VMEM((B, W2S, LANE, LANE), F32),
            pltpu.SemaphoreType.DMA((N_SEM,)),
        ],
        compiler_params=pltpu.CompilerParams(vmem_limit_bytes=100 * 1024 * 1024,
                                             disable_semaphore_checks=True,
                                             disable_bounds_checks=True),
    )(x2, kt, vt, wq, wo, w1, w3, w2)
    return out.reshape(B, Sq, D)
```

```python
import jax
import jax.numpy as jnp
from jax import lax
import jax.experimental.pallas as pl
import jax.experimental.pallas.tpu as pltpu

F32 = jnp.float32
BF16 = jnp.bfloat16
A = slice(None)

HQ = 32
DH = 192
LANE = 128
RA = 32
NJ = RA // 8
AH = DH // RA
HG = 4
GROWS = HG * DH
LEAD = 16
UNROLL = 4
LA = 4

VD = (3, 4, 2)
BIG = (A, A, A)
SMALL = [(A, e, r) for e in range(4) for r in range(2)]
ORDER = (("v", 0, BIG), ("v", 1, BIG), ("k", 0, BIG), ("v", 2, BIG), ("v", 3, BIG), ("k", 2, BIG),
         ("k", 3, (A, A, 0)), ("k", 3, (A, A, 1)))
T0 = [("k", 1, s, c) for s in SMALL for c in range(16)]
T1 = [o + (c,) for o in ORDER for c in range(16)]
FIRST = [(("k", 2 * u, BIG, c), ("k", 2 * u + 1, BIG, c)) for u in range(2) for c in range(16)]
LAST_COLS = (2, 2, 2, 2)
UL = 16


def _zip(t0, t1):
    n = max(len(t0), len(t1))
    pick = lambda t, i: t[i * len(t) // n] if (i + 1) * len(t) // n > i * len(t) // n else None
    return [(pick(t0, i), pick(t1, i)) for i in range(n)]


_PAIRS = _zip(T0, T1)
NU = round(len(_PAIRS) / UL)
UNITS = [_PAIRS[u * UL:(u + 1) * UL if u < NU - 1 else None] for u in range(NU)]
DONE = {}
for _key in [("v", _j) for _j in range(NJ)] + [("k", None)]:
    _u = max(_i for _i, _un in enumerate(UNITS) for _p in _un for _d in _p
             if _d and _d[0] == _key[0] and _key[1] in (None, _d[1]))
    DONE.setdefault(_u, []).append(_key)

W2S = 4
W2_MAIN = 24
W2_SMALL = 3
TAIL_GRAN = (3, 3, 2, 2, 1, 1)
LAST_ISSUE = 16

X_SEM, Q_SEM, F1_SEM, F2_SEM, O_SEM, K_SEM, V_SEM = 0, 1, 2, 3, 4, 5, 7
T_SEM = V_SEM + 2 * NJ
N_SEM = T_SEM + len(TAIL_GRAN)


def _kernel(x_hbm, k_hbm, v_hbm, wq_hbm, wo_hbm, w1_hbm, w3_hbm, w2_hbm,
            out_ref,
            x_v, wq_v, wo_v, w1_v, w3_v, w2_v, kbuf, vbuf, qblk, p_s, acc, h_s, hb_s,
            sems, *, B, D, S, W, F):
    NC = W // LANE
    GPB = HQ // HG
    NG = B * GPB
    S0 = S - W
    FS = F // W2S

    def rows8(j):
        return pl.ds(j * 8, 8) if isinstance(j, int) else pl.ds(pl.multiple_of(j * 8, 8), 8)

    def lanes(c, m=1, off=0):
        n = m * LANE
        if isinstance(c, int):
            return pl.ds(off + c * n, n)
        return pl.ds(pl.multiple_of(off + c * n, LANE), n)

    def k_copy(g, j, sel, c):
        slot = g % 2
        return pltpu.make_async_copy(
            k_hbm.at[(g, *sel, rows8(j), lanes(c, 1, S0))],
            kbuf.at[(slot, *sel, rows8(j), lanes(c))],
            sems.at[K_SEM + slot])

    def v_copy(g, j, sel, c):
        slot = (g % 2) * NJ + j
        return pltpu.make_async_copy(
            v_hbm.at[(g, *sel, j, A, lanes(c, 1, S0))],
            vbuf.at[(slot, *sel, A, lanes(c))],
            sems.at[V_SEM + slot])

    def wait_all(buf, sem):
        pltpu.make_async_copy(buf, buf, sems.at[sem]).wait()

    def w_copy(src, dst, idx, sem):
        return pltpu.make_async_copy(src.at[idx], dst.at[idx], sems.at[sem])

    def loop(lo, hi, fn, unroll=1):
        def body(i, carry):
            fn(i)
            return carry
        lax.fori_loop(lo, hi, body, 0, unroll=unroll)

    def issue_w13(j):
        for c in range(F // (4 * LANE)):
            w_copy(w1_hbm, w1_v, (A, rows8(j), lanes(c, 4)), F1_SEM).start(priority=0)
            w_copy(w3_hbm, w3_v, (A, rows8(j), lanes(c, 4)), F1_SEM).start(priority=1)

    def issue_w2(j):
        w_copy(w2_hbm, w2_v, (A, rows8(j), A), F2_SEM).start(priority=0)
        w_copy(w2_hbm, w2_v, (A, rows8(j + W2_MAIN // 2), A), F2_SEM).start(priority=1)

    def issue_wo(j):
        w_copy(wo_hbm, wo_v, (pl.ds(0, 4), j), O_SEM).start(priority=0)
        w_copy(wo_hbm, wo_v, (pl.ds(4, 4), j), O_SEM).start(priority=1)

    def issue_unit(g, unit):
        for pair in unit:
            for prio, d in enumerate(pair):
                if d is not None:
                    cp = k_copy(g + 1, *d[1:]) if d[0] == "k" else v_copy(g, *d[1:])
                    cp.start(priority=prio)

    W2_TAIL = FS // 8 - sum(TAIL_GRAN)
    tail_sem = {j: F2_SEM for j in range(W2_MAIN, W2_TAIL)}
    for t, n in enumerate(TAIL_GRAN):
        for _ in range(n):
            tail_sem[W2_MAIN + len(tail_sem)] = T_SEM + t
    t0_list, t1_list = [], []
    for j, c0 in enumerate(LAST_COLS):
        t0_list += [(j, sel, c) for sel in SMALL for c in range(c0)]
        t1_list += [(j, BIG, c) for c in range(c0, NC)]
    t0_list += [(a, j) for j in range(W2_MAIN, W2_MAIN + W2_SMALL) for a in range(W2S)]
    t1_list += [(A, j) for j in range(W2_MAIN + W2_SMALL, FS // 8)]
    n_last = max(len(t0_list), len(t1_list))

    def issue_last(lo, hi):
        for i in range(lo, min(hi, n_last)):
            for prio, lst in enumerate((t0_list, t1_list)):
                if i >= len(lst):
                    continue
                d = lst[i]
                if len(d) == 2:
                    cp = w_copy(w2_hbm, w2_v, (d[0], rows8(d[1]), A), tail_sem[d[1]])
                else:
                    cp = v_copy(NG - 1, *d)
                cp.start(priority=prio)

    def qproj(xn, hg):
        w = wq_v[:, :, hg * GROWS:(hg + 1) * GROWS].reshape(D, GROWS)
        q = jnp.dot(xn, w, preferred_element_type=F32).astype(BF16).astype(F32)
        row = lax.broadcasted_iota(jnp.int32, (8, GROWS), 0)
        col = lax.broadcasted_iota(jnp.int32, (8, GROWS), 1)
        diag = (col >= row * DH) & (col < (row + 1) * DH)
        for b in range(B):
            qb = jnp.broadcast_to(q[b:b + 1, :], (8, GROWS))
            qblk[b * GPB + hg] = jnp.where(diag, qb, 0.0)

    def scores_softmax(g):
        slot = g % 2
        wait_all(kbuf.at[slot], K_SEM + slot)
        kk = kbuf[slot].reshape(GROWS, W)
        s = jnp.dot(qblk[g].astype(BF16), kk, preferred_element_type=F32) * (DH ** -0.5)
        m = jnp.max(s, axis=-1, keepdims=True)
        e = jnp.exp(s - m)
        l = jnp.sum(e, axis=-1, keepdims=True)
        p_s[slot] = e * (1.0 / l)

    def pv_wo(g, j):
        slot = (g % 2) * NJ + j
        wait_all(vbuf.at[slot], V_SEM + slot)
        b, hg = g // GPB, g % GPB
        tot = acc[b]
        for hh in range(HG):
            pb = jnp.broadcast_to(p_s[g % 2, hh:hh + 1, :], (8, W))
            for a in range(hh * AH, (hh + 1) * AH):
                ai = (a // (VD[1] * VD[2]), a // VD[2] % VD[1], a % VD[2])
                prod = vbuf[(slot, *ai)].astype(F32) * pb
                o = jnp.sum(prod, axis=-1, keepdims=True)
                tot = tot + o * wo_v[hg, NJ * a + j].astype(F32)
        acc[b] = tot

    def consume(g, u):
        for which, j in DONE.get(u, ()):
            if which == "k":
                scores_softmax(g + 1)
            elif not (isinstance(g, int) and g < 0):
                pv_wo(g, j)

    def ffn_down(lo, hi):
        lo, hi = lo * 8, hi * 8
        wait_all(w2_v.at[:, pl.ds(lo, hi - lo)], F2_SEM)
        out = None
        for a in range(W2S):
            part = jnp.dot(h_s[:, a * FS + lo:a * FS + hi].astype(BF16), w2_v[a, lo:hi, :],
                           preferred_element_type=F32)
            out = part if out is None else out + part
        return out

    def in_row0(v, b):
        row8 = lax.broadcasted_iota(jnp.int32, (8, D), 0)
        return jnp.where(row8 == 0, jnp.broadcast_to(v[b:b + 1, :], (8, D)), 0.0)

    wq_descs = [(A, rows8(j), lanes(c, 4))
                for j in range(16) for c in range(HQ * DH // (4 * LANE))]
    n0 = (len(wq_descs) - LEAD) // 2
    for i in range(LEAD):
        w_copy(wq_hbm, wq_v, wq_descs[n0 + i], Q_SEM).start(priority=1)
    xcp = pltpu.make_async_copy(x_hbm, x_v, sems.at[X_SEM])
    xcp.start()
    for i in range(n0):
        w_copy(wq_hbm, wq_v, wq_descs[i], Q_SEM).start(priority=0)
        w_copy(wq_hbm, wq_v, wq_descs[n0 + LEAD + i], Q_SEM).start(priority=1)
    xcp.wait()
    x = x_v[...].astype(F32)
    mu = jnp.mean(x, axis=-1, keepdims=True)
    xc = x - mu
    var = jnp.mean(xc * xc, axis=-1, keepdims=True)
    xn4 = xc / jnp.sqrt(var + 1e-5)
    xn = jnp.concatenate([xn4, jnp.zeros((8 - B, D), F32)], axis=0).astype(BF16)
    loop(0, 16, issue_w13)
    wait_all(wq_v, Q_SEM)
    for hg in range(GPB // 2):
        qproj(xn, hg)
    loop(0, W2_MAIN // 2, issue_w2)
    loop(0, 16, issue_wo)
    for hg in range(GPB // 2, GPB):
        qproj(xn, hg)
    loop(16, 40, issue_wo)
    wait_all(w1_v, F1_SEM)
    wait_all(w3_v, F1_SEM)
    gate = jnp.dot(xn, w1_v[...].reshape(D, F), preferred_element_type=F32)
    up = jnp.dot(xn, w3_v[...].reshape(D, F), preferred_element_type=F32)
    h_s[...] = (gate * jax.nn.sigmoid(gate) * up).astype(BF16).astype(F32)
    loop(40, 64, issue_wo)
    base = x + ffn_down(0, W2_MAIN)[0:B, :]
    for b in range(B):
        acc[b] = in_row0(base, b)
    eye = (lax.broadcasted_iota(jnp.int32, (LANE, LANE), 0)
           == lax.broadcasted_iota(jnp.int32, (LANE, LANE), 1))
    for b in range(B):
        for a in range(W2S):
            hrow = h_s[b:b + 1, (a + 1) * FS - LANE:(a + 1) * FS]
            col = jnp.sum(jnp.where(eye, jnp.broadcast_to(hrow, (LANE, LANE)), 0.0),
                          axis=-1, keepdims=True)
            hb_s[b, a] = jnp.broadcast_to(col, (LANE, LANE))
    loop(64, 96, issue_wo)
    issue_unit(-1, FIRST)
    wait_all(wo_v, O_SEM)
    for u in range(LA):
        issue_unit(0, UNITS[u])
    scores_softmax(0)

    def step(g, issue_next):
        for u in range(NU):
            if u + LA < NU:
                issue_unit(g, UNITS[u + LA])
            else:
                issue_next(u + LA - NU)
            consume(g, u)

    def group_body(g, carry):
        step(g, lambda u: issue_unit(g + 1, UNITS[u]))
        return carry

    lax.fori_loop(0, NG - 2, group_body, 0)

    step(NG - 2, lambda u: issue_last(u * LAST_ISSUE, (u + 1) * LAST_ISSUE))
    issue_last(LA * LAST_ISSUE, n_last)
    for j in range(NJ):
        pv_wo(NG - 1, j)
    tot = [acc[b] for b in range(B)]
    mid = ffn_down(W2_MAIN, W2_TAIL)
    tot = [tot[b] + in_row0(mid, b) for b in range(B)]
    j0 = W2_TAIL
    for t, n in enumerate(TAIL_GRAN):
        wait_all(w2_v.at[:, pl.ds(j0 * 8, n * 8)], T_SEM + t)
        for j in range(j0, j0 + n):
            for a in range(W2S):
                wrow = w2_v[a, j * 8:j * 8 + 8, :].astype(F32)
                r = j * 8 - (FS - LANE)
                for b in range(B):
                    hb = hb_s[b, a, r:r + 8, :]
                    tot[b] = tot[b] + jnp.concatenate([hb] * (D // LANE), axis=1) * wrow
        j0 += n
    res = jnp.concatenate([jnp.sum(t, axis=0, keepdims=True) for t in tot], axis=0)
    out_ref[...] = res.astype(out_ref.dtype)


@jax.jit
def pallas_parallel_sum__sliding_block_cached__glu_gated_swiglu__decode_kernel(
    A_x: jax.Array,
    A_k_cache: jax.Array,
    A_v_cache: jax.Array,
    A_wq: jax.Array,
    A_wo: jax.Array,
    B_x: jax.Array,
    B_w1: jax.Array,
    B_w3: jax.Array,
    B_w2: jax.Array,
):
    B, Sq, D = A_x.shape
    _, Hkv, S, Dh = A_k_cache.shape
    F = B_w1.shape[1]
    assert (B, Sq, D, Hkv, Dh, F) == (4, 1, 640, HQ, DH, 1536)
    W = min(4096, max(256, S // 4))
    assert W == 2048 and sum(TAIL_GRAN) * 8 <= LANE
    NG = B * HQ // HG

    kt = jnp.swapaxes(A_k_cache, 2, 3).reshape(NG, *VD, RA, S)
    vt = jnp.swapaxes(A_v_cache, 2, 3).reshape(NG, *VD, NJ, 8, S)
    x2 = A_x.reshape(B, D)
    wq = A_wq.reshape(5, D // 5, HQ * DH)
    wo = A_wo.reshape(HQ // HG, GROWS // 8, 8, D)
    w1 = B_w1.reshape(5, D // 5, F)
    w3 = B_w3.reshape(5, D // 5, F)
    w2 = B_w2.reshape(W2S, F // W2S, D)

    kern = lambda *refs: _kernel(*refs, B=B, D=D, S=S, W=W, F=F)
    out = pl.pallas_call(
        kern,
        in_specs=[pl.BlockSpec(memory_space=pl.ANY)] * 8,
        out_specs=pl.BlockSpec(memory_space=pltpu.VMEM),
        out_shape=jax.ShapeDtypeStruct((B, D), A_x.dtype),
        scratch_shapes=[
            pltpu.VMEM((B, D), BF16),
            pltpu.VMEM(wq.shape, BF16),
            pltpu.VMEM(wo.shape, BF16),
            pltpu.VMEM(w1.shape, BF16),
            pltpu.VMEM(w3.shape, BF16),
            pltpu.VMEM(w2.shape, BF16),
            pltpu.VMEM((2, *VD, RA, W), BF16),
            pltpu.VMEM((2 * NJ, *VD, 8, W), BF16),
            pltpu.VMEM((NG, 8, GROWS), F32),
            pltpu.VMEM((2, 8, W), F32),
            pltpu.VMEM((B, 8, D), F32),
            pltpu.VMEM((8, F), F32),
            pltpu.VMEM((B, W2S, LANE, LANE), F32),
            pltpu.SemaphoreType.DMA((N_SEM,)),
        ],
        compiler_params=pltpu.CompilerParams(vmem_limit_bytes=100 * 1024 * 1024,
                                             disable_semaphore_checks=True,
                                             disable_bounds_checks=True),
    )(x2, kt, vt, wq, wo, w1, w3, w2)
    return out.reshape(B, Sq, D)
```

```python
import jax
import jax.numpy as jnp
from jax import lax
import jax.experimental.pallas as pl
import jax.experimental.pallas.tpu as pltpu

F32 = jnp.float32
BF16 = jnp.bfloat16
A = slice(None)

HQ = 32
DH = 192
LANE = 128
RA = 32
NJ = RA // 8
AH = DH // RA
HG = 4
SHIFT = 2
GROWS = HG * DH
LEAD = 24
LA = 3

NA = HG * AH
BREV = (0, 4, 2, 6, 1, 5, 3, 7)
JROT = 0


def _block(which, j, blk):
    return [(which, j, 8 * blk + x) for x in BREV]


def _slice(which, j):
    return [d for blk in range(NA // 8) for d in _block(which, j, blk)]


UNITS = [list(zip(_slice("k", (j + JROT) % NJ), _slice("v", j))) for j in range(NJ)]
FIRST = list(zip(_slice("k", 0) + _slice("k", 1), _slice("k", 2) + _slice("k", 3)))
LAST0 = ((0, 0), (0, 1), (0, 2), (1, 1), (2, 0), (2, 2), (3, 1))
LAST1 = ((1, 0), (1, 2), (2, 1), (3, 0), (3, 2))
DONE = {0: [("v", 0)], 1: [("v", 1)], 2: [("v", 2)], 3: [("k", None), ("v", 3)]}
NU = len(UNITS)

W2S = 4
W2_MAIN = 24
W2_T0 = 4
TAIL_GRAN = (3, 3, 2, 2, 1, 1)
LAST_ISSUE = 20

X_SEM, Q_SEM, F1_SEM, F3_SEM, F2_SEM, O_SEM, K_SEM, V_SEM = 0, 1, 2, 3, 4, 5, 6, 8
T_SEM = V_SEM + 2 * NJ
N_SEM = T_SEM + len(TAIL_GRAN)


def _kernel(x_hbm, k_hbm, v_hbm, wq_hbm, wo_hbm, w1_hbm, w3_hbm, w2_hbm,
            out_ref,
            x_v, wq_v, wo_v, w1_v, w3_v, w2_v, kbuf, vbuf, qblk, p_s, acc, h_s, hb_s,
            sems, *, B, D, S, W, F):
    NC = W // LANE
    GPB = HQ // HG
    NG = B * GPB
    S0 = S - W
    FS = F // W2S

    def rows8(j):
        return pl.ds(j * 8, 8) if isinstance(j, int) else pl.ds(pl.multiple_of(j * 8, 8), 8)

    def lanes(c, m=1, off=0):
        n = m * LANE
        if isinstance(c, int):
            return pl.ds(off + c * n, n)
        return pl.ds(pl.multiple_of(off + c * n, LANE), n)

    def a_glob(g, a):
        lo = g * NA - SHIFT * AH
        if a >= SHIFT * AH:
            return lo + a
        if isinstance(g, int):
            return (lo + a) % (B * HQ * AH)
        return jnp.where(g == 0, B * HQ * AH - SHIFT * AH, lo) + a

    def k_copy(g, j, a):
        slot = g % 2
        return pltpu.make_async_copy(k_hbm.at[a_glob(g, a), rows8(j), pl.ds(S0, W)],
                                     kbuf.at[slot, a, rows8(j)], sems.at[K_SEM + slot])

    def v_copy(g, j, a):
        slot = (g % 2) * NJ + j
        return pltpu.make_async_copy(v_hbm.at[a_glob(g, a), rows8(j), pl.ds(S0, W)],
                                     vbuf.at[slot, a], sems.at[V_SEM + slot])

    def wait_all(buf, sem):
        pltpu.make_async_copy(buf, buf, sems.at[sem]).wait()

    def w_copy(src, dst, idx, sem):
        return pltpu.make_async_copy(src.at[idx], dst.at[idx], sems.at[sem])

    def loop(lo, hi, fn, unroll=1):
        def body(i, carry):
            fn(i)
            return carry
        lax.fori_loop(lo, hi, body, 0, unroll=unroll)

    def issue_w13(j):
        for c in range(F // (4 * LANE)):
            w_copy(w1_hbm, w1_v, (A, rows8(j), lanes(c, 4)), F1_SEM).start(priority=0)
            w_copy(w3_hbm, w3_v, (A, rows8(j), lanes(c, 4)), F3_SEM).start(priority=1)

    def issue_w2(j):
        w_copy(w2_hbm, w2_v, (A, rows8(j), A), F2_SEM).start(priority=0)
        w_copy(w2_hbm, w2_v, (A, rows8(j + W2_MAIN // 2), A), F2_SEM).start(priority=1)

    def issue_wo(j):
        w_copy(wo_hbm, wo_v, (pl.ds(0, 4), j), O_SEM).start(priority=0)
        w_copy(wo_hbm, wo_v, (pl.ds(4, 4), j), O_SEM).start(priority=1)

    def issue_unit(g, unit):
        for pair in unit:
            for prio, d in enumerate(pair):
                if d is not None:
                    cp = k_copy(g + 1, *d[1:]) if d[0] == "k" else v_copy(g, *d[1:])
                    cp.start(priority=prio)

    W2_TAIL = FS // 8 - sum(TAIL_GRAN)
    tail_sem = {j: F2_SEM for j in range(W2_MAIN, W2_TAIL)}
    for t, n in enumerate(TAIL_GRAN):
        for _ in range(n):
            tail_sem[W2_MAIN + len(tail_sem)] = T_SEM + t
    t0_list = [d for j, blk in LAST0 for d in _block("v", j, blk)]
    t1_list = [d for j, blk in LAST1 for d in _block("v", j, blk)]
    t0_list += [("w2", j) for j in range(W2_MAIN, W2_MAIN + W2_T0)]
    t1_list += [("w2", j) for j in range(W2_MAIN + W2_T0, FS // 8)]
    n_last = max(len(t0_list), len(t1_list))

    def issue_last(lo, hi):
        for i in range(lo, min(hi, n_last)):
            for prio, lst in enumerate((t0_list, t1_list)):
                if i >= len(lst):
                    continue
                d = lst[i]
                if d[0] == "w2":
                    cp = w_copy(w2_hbm, w2_v, (A, rows8(d[1]), A), tail_sem[d[1]])
                else:
                    cp = v_copy(NG - 1, *d[1:])
                cp.start(priority=prio)

    HALF = GROWS // 2

    def qproj(xn, hg):
        w = wq_v[:, :, hg * GROWS:(hg + 1) * GROWS].reshape(D, GROWS)
        q = jnp.dot(xn, w, preferred_element_type=F32).astype(BF16).astype(F32)
        row = lax.broadcasted_iota(jnp.int32, (8, HALF), 0)
        col = lax.broadcasted_iota(jnp.int32, (8, HALF), 1)
        for b in range(B):
            for hf in range(2):
                g, pos = divmod((2 * (b * GPB + hg) + hf + SHIFT // 2) % (2 * NG), 2)
                diag = (col >= (row - 2 * pos) * DH) & (col < (row - 2 * pos + 1) * DH)
                qb = jnp.broadcast_to(q[b:b + 1, hf * HALF:(hf + 1) * HALF], (8, HALF))
                qblk[g, :, pos * HALF:(pos + 1) * HALF] = jnp.where(diag, qb, 0.0)

    def scores_softmax(g):
        slot = g % 2
        wait_all(kbuf.at[slot], K_SEM + slot)
        kk = kbuf[slot].reshape(GROWS, W)
        s = jnp.dot(qblk[g].astype(BF16), kk, preferred_element_type=F32) * (DH ** -0.5)
        m = jnp.max(s, axis=-1, keepdims=True)
        e = jnp.exp(s - m)
        l = jnp.sum(e, axis=-1, keepdims=True)
        p_s[slot] = e * (1.0 / l)

    def pv_wo(g, j):
        slot = (g % 2) * NJ + j
        wait_all(vbuf.at[slot], V_SEM + slot)
        for pos in range(2):
            hf = (pos + SHIFT // 2) % 2
            gu = g if pos >= SHIFT // 2 else (g + NG - 1) % NG
            b, hg = gu // GPB, gu % GPB
            tot = acc[b]
            for hh in range(2):
                pb = jnp.broadcast_to(p_s[g % 2, 2 * pos + hh:2 * pos + hh + 1, :], (8, W))
                for i in range(hh * AH, (hh + 1) * AH):
                    a = pos * 2 * AH + i
                    prod = vbuf[slot, a].astype(F32) * pb
                    o = jnp.sum(prod, axis=-1, keepdims=True)
                    tot = tot + o * wo_v[hg, NJ * (hf * 2 * AH + i) + j].astype(F32)
            acc[b] = tot

    def consume(g, u):
        for which, j in DONE.get(u, ()):
            if which == "k":
                scores_softmax(g + 1)
            elif not (isinstance(g, int) and g < 0):
                pv_wo(g, j)

    def ffn_down(lo, hi):
        lo, hi = lo * 8, hi * 8
        wait_all(w2_v.at[:, pl.ds(lo, hi - lo)], F2_SEM)
        out = None
        for a in range(W2S):
            part = jnp.dot(h_s[:, a * FS + lo:a * FS + hi].astype(BF16), w2_v[a, lo:hi, :],
                           preferred_element_type=F32)
            out = part if out is None else out + part
        return out

    def in_row0(v, b):
        row8 = lax.broadcasted_iota(jnp.int32, (8, D), 0)
        return jnp.where(row8 == 0, jnp.broadcast_to(v[b:b + 1, :], (8, D)), 0.0)

    wq_descs = [(A, rows8(j), lanes(c, 4))
                for j in range(16) for c in range(HQ * DH // (4 * LANE))]
    n0 = (len(wq_descs) - LEAD) // 2
    for i in range(LEAD):
        w_copy(wq_hbm, wq_v, wq_descs[n0 + i], Q_SEM).start(priority=1)
    xcp = pltpu.make_async_copy(x_hbm, x_v, sems.at[X_SEM])
    xcp.start()
    for i in range(n0):
        w_copy(wq_hbm, wq_v, wq_descs[i], Q_SEM).start(priority=0)
        w_copy(wq_hbm, wq_v, wq_descs[n0 + LEAD + i], Q_SEM).start(priority=1)
    xcp.wait()
    x = x_v[...].astype(F32)
    mu = jnp.mean(x, axis=-1, keepdims=True)
    xc = x - mu
    var = jnp.mean(xc * xc, axis=-1, keepdims=True)
    xn4 = xc / jnp.sqrt(var + 1e-5)
    xn = jnp.concatenate([xn4, jnp.zeros((8 - B, D), F32)], axis=0).astype(BF16)
    loop(0, 16, issue_w13)
    wait_all(wq_v, Q_SEM)
    for hg in range(GPB // 2):
        qproj(xn, hg)
    loop(0, W2_MAIN // 2, issue_w2)
    loop(0, 16, issue_wo)
    for hg in range(GPB // 2, GPB):
        qproj(xn, hg)
    loop(16, 40, issue_wo)
    wait_all(w1_v, F1_SEM)
    wait_all(w3_v, F3_SEM)
    gate = jnp.dot(xn, w1_v[...].reshape(D, F), preferred_element_type=F32)
    up = jnp.dot(xn, w3_v[...].reshape(D, F), preferred_element_type=F32)
    h_s[...] = (gate * jax.nn.sigmoid(gate) * up).astype(BF16).astype(F32)
    loop(40, 64, issue_wo)
    base = x + ffn_down(0, W2_MAIN)[0:B, :]
    for b in range(B):
        acc[b] = in_row0(base, b)
    eye = (lax.broadcasted_iota(jnp.int32, (LANE, LANE), 0)
           == lax.broadcasted_iota(jnp.int32, (LANE, LANE), 1))
    for b in range(B):
        for a in range(W2S):
            hrow = h_s[b:b + 1, (a + 1) * FS - LANE:(a + 1) * FS]
            col = jnp.sum(jnp.where(eye, jnp.broadcast_to(hrow, (LANE, LANE)), 0.0),
                          axis=-1, keepdims=True)
            hb_s[b, a] = jnp.broadcast_to(col, (LANE, LANE))
    loop(64, 96, issue_wo)
    issue_unit(-1, FIRST)
    wait_all(wo_v, O_SEM)
    for u in range(LA):
        issue_unit(0, UNITS[u])
    scores_softmax(0)

    def step(g, issue_next):
        for u in range(NU):
            if u + LA < NU:
                issue_unit(g, UNITS[u + LA])
            else:
                issue_next(u + LA - NU)
            consume(g, u)

    def group_body(g, carry):
        step(g, lambda u: issue_unit(g + 1, UNITS[u]))
        return carry

    lax.fori_loop(0, NG - 2, group_body, 0)

    step(NG - 2, lambda u: issue_last(u * LAST_ISSUE, (u + 1) * LAST_ISSUE))
    issue_last(LA * LAST_ISSUE, n_last)
    for j in range(NJ):
        pv_wo(NG - 1, j)
    tot = [acc[b] for b in range(B)]
    mid = ffn_down(W2_MAIN, W2_TAIL)
    tot = [tot[b] + in_row0(mid, b) for b in range(B)]
    j0 = W2_TAIL
    for t, n in enumerate(TAIL_GRAN):
        wait_all(w2_v.at[:, pl.ds(j0 * 8, n * 8)], T_SEM + t)
        for j in range(j0, j0 + n):
            for a in range(W2S):
                wrow = w2_v[a, j * 8:j * 8 + 8, :].astype(F32)
                r = j * 8 - (FS - LANE)
                for b in range(B):
                    hb = hb_s[b, a, r:r + 8, :]
                    tot[b] = tot[b] + jnp.concatenate([hb] * (D // LANE), axis=1) * wrow
        j0 += n
    res = jnp.concatenate([jnp.sum(t, axis=0, keepdims=True) for t in tot], axis=0)
    out_ref[...] = res.astype(out_ref.dtype)


@jax.jit
def pallas_parallel_sum__sliding_block_cached__glu_gated_swiglu__decode_kernel(
    A_x: jax.Array,
    A_k_cache: jax.Array,
    A_v_cache: jax.Array,
    A_wq: jax.Array,
    A_wo: jax.Array,
    B_x: jax.Array,
    B_w1: jax.Array,
    B_w3: jax.Array,
    B_w2: jax.Array,
):
    B, Sq, D = A_x.shape
    _, Hkv, S, Dh = A_k_cache.shape
    F = B_w1.shape[1]
    assert (B, Sq, D, Hkv, Dh, F) == (4, 1, 640, HQ, DH, 1536)
    W = min(4096, max(256, S // 4))
    assert W == 2048 and sum(TAIL_GRAN) * 8 <= LANE
    NG = B * HQ // HG

    kt = jnp.swapaxes(A_k_cache, 2, 3).reshape(B * HQ * AH, RA, S)
    vt = jnp.swapaxes(A_v_cache, 2, 3).reshape(B * HQ * AH, RA, S)
    x2 = A_x.reshape(B, D)
    wq = A_wq.reshape(5, D // 5, HQ * DH)
    wo = A_wo.reshape(HQ // HG, GROWS // 8, 8, D)
    w1 = B_w1.reshape(5, D // 5, F)
    w3 = B_w3.reshape(5, D // 5, F)
    w2 = B_w2.reshape(W2S, F // W2S, D)

    kern = lambda *refs: _kernel(*refs, B=B, D=D, S=S, W=W, F=F)
    out = pl.pallas_call(
        kern,
        in_specs=[pl.BlockSpec(memory_space=pl.ANY)] * 8,
        out_specs=pl.BlockSpec(memory_space=pltpu.VMEM),
        out_shape=jax.ShapeDtypeStruct((B, D), A_x.dtype),
        scratch_shapes=[
            pltpu.VMEM((B, D), BF16),
            pltpu.VMEM(wq.shape, BF16),
            pltpu.VMEM(wo.shape, BF16),
            pltpu.VMEM(w1.shape, BF16),
            pltpu.VMEM(w3.shape, BF16),
            pltpu.VMEM(w2.shape, BF16),
            pltpu.VMEM((2, NA, RA, W), BF16),
            pltpu.VMEM((2 * NJ, NA, 8, W), BF16),
            pltpu.VMEM((NG, 8, GROWS), F32),
            pltpu.VMEM((2, 8, W), F32),
            pltpu.VMEM((B, 8, D), F32),
            pltpu.VMEM((8, F), F32),
            pltpu.VMEM((B, W2S, LANE, LANE), F32),
            pltpu.SemaphoreType.DMA((N_SEM,)),
        ],
        compiler_params=pltpu.CompilerParams(vmem_limit_bytes=100 * 1024 * 1024,
                                             disable_semaphore_checks=True,
                                             disable_bounds_checks=True),
    )(x2, kt, vt, wq, wo, w1, w3, w2)
    return out.reshape(B, Sq, D)
```

```python
import jax
import jax.numpy as jnp
from jax import lax
import jax.experimental.pallas as pl
import jax.experimental.pallas.tpu as pltpu

F32 = jnp.float32
BF16 = jnp.bfloat16
A = slice(None)

HQ = 32
DH = 192
LANE = 128
RH = DH // 8
HG = 4
SHIFT = 2
GROWS = HG * DH
LEAD = 24
LA = 3

RG = GROWS // 8
SEQ32 = [8 * x + y for y in (0, 1, 4, 5, 2, 3, 6, 7) for x in (0, 3, 1, 2)]
SEQ = [32 * blk + r for blk in range(RG // 32) for r in SEQ32]
NU = 4
UL = RG // NU
FIRST = (SEQ[:RG // 2], SEQ[RG // 2:])
LAST0 = (0, 1, 2, 4, 6, 8, 10)
LAST1 = (3, 5, 7, 9, 11)

W2S = 4
W2_MAIN = 24
W2_T0 = 4
TAIL_GRAN = (3, 3, 2, 2, 1, 1)
LAST_ISSUE = 20

X_SEM, Q_SEM, F1_SEM, F3_SEM, F2_SEM, O_SEM, K_SEM, V_SEM = 0, 1, 2, 3, 4, 5, 6, 8
T_SEM = V_SEM + 2 * NU
N_SEM = T_SEM + len(TAIL_GRAN)


def _kernel(x_hbm, k_hbm, v_hbm, wq_hbm, wo_hbm, w1_hbm, w3_hbm, w2_hbm,
            out_ref,
            x_v, wq_v, wo_v, w1_v, w3_v, w2_v, kbuf, vbuf, qblk, p_s, acc, h_s, hb_s,
            sems, *, B, D, S, W, F):
    NC = W // LANE
    GPB = HQ // HG
    NG = B * GPB
    S0 = S - W
    FS = F // W2S

    def rows8(j):
        return pl.ds(j * 8, 8) if isinstance(j, int) else pl.ds(pl.multiple_of(j * 8, 8), 8)

    def lanes(c, m=1, off=0):
        n = m * LANE
        if isinstance(c, int):
            return pl.ds(off + c * n, n)
        return pl.ds(pl.multiple_of(off + c * n, LANE), n)

    def head_of(g, r):
        lo = g * HG - SHIFT
        hh = r // RH
        if hh >= SHIFT:
            return lo + hh
        if isinstance(g, int):
            return (lo + hh) % (B * HQ)
        return jnp.where(g == 0, B * HQ - SHIFT, lo) + hh

    def k_copy(g, r):
        slot = g % 2
        return pltpu.make_async_copy(k_hbm.at[head_of(g, r), rows8(r % RH), pl.ds(S0, W)],
                                     kbuf.at[slot, rows8(r)], sems.at[K_SEM + slot])

    def v_copy(g, pos):
        slot = (g % 2) * NU + pos // UL
        r = SEQ[pos]
        return pltpu.make_async_copy(v_hbm.at[head_of(g, r), rows8(r % RH), pl.ds(S0, W)],
                                     vbuf.at[slot, pos % UL], sems.at[V_SEM + slot])

    def wait_all(buf, sem):
        pltpu.make_async_copy(buf, buf, sems.at[sem]).wait()

    def w_copy(src, dst, idx, sem):
        return pltpu.make_async_copy(src.at[idx], dst.at[idx], sems.at[sem])

    def loop(lo, hi, fn, unroll=1):
        def body(i, carry):
            fn(i)
            return carry
        lax.fori_loop(lo, hi, body, 0, unroll=unroll)

    def issue_w13(j):
        for c in range(F // (4 * LANE)):
            w_copy(w1_hbm, w1_v, (A, rows8(j), lanes(c, 4)), F1_SEM).start(priority=0)
            w_copy(w3_hbm, w3_v, (A, rows8(j), lanes(c, 4)), F3_SEM).start(priority=1)

    def issue_w2(j):
        w_copy(w2_hbm, w2_v, (A, rows8(j), A), F2_SEM).start(priority=0)
        w_copy(w2_hbm, w2_v, (A, rows8(j + W2_MAIN // 2), A), F2_SEM).start(priority=1)

    def issue_wo(j):
        w_copy(wo_hbm, wo_v, (pl.ds(0, 4), j), O_SEM).start(priority=0)
        w_copy(wo_hbm, wo_v, (pl.ds(4, 4), j), O_SEM).start(priority=1)

    def issue_unit(g, u):
        for pos in range(u * UL, (u + 1) * UL):
            k_copy(g + 1, SEQ[pos]).start(priority=0)
            v_copy(g, pos).start(priority=1)

    W2_TAIL = FS // 8 - sum(TAIL_GRAN)
    tail_sem = {j: F2_SEM for j in range(W2_MAIN, W2_TAIL)}
    for t, n in enumerate(TAIL_GRAN):
        for _ in range(n):
            tail_sem[W2_MAIN + len(tail_sem)] = T_SEM + t
    t0_list = [("v", 8 * ch + i) for ch in LAST0 for i in range(8)]
    t1_list = [("v", 8 * ch + i) for ch in LAST1 for i in range(8)]
    t0_list += [("w2", j) for j in range(W2_MAIN, W2_MAIN + W2_T0)]
    t1_list += [("w2", j) for j in range(W2_MAIN + W2_T0, FS // 8)]
    n_last = max(len(t0_list), len(t1_list))

    def issue_last(lo, hi):
        for i in range(lo, min(hi, n_last)):
            for prio, lst in enumerate((t0_list, t1_list)):
                if i >= len(lst):
                    continue
                d = lst[i]
                if d[0] == "w2":
                    cp = w_copy(w2_hbm, w2_v, (A, rows8(d[1]), A), tail_sem[d[1]])
                else:
                    cp = v_copy(NG - 1, d[1])
                cp.start(priority=prio)

    HALF = GROWS // 2

    def qproj(xn, hg):
        w = wq_v[:, :, hg * GROWS:(hg + 1) * GROWS].reshape(D, GROWS)
        q = jnp.dot(xn, w, preferred_element_type=F32).astype(BF16).astype(F32)
        row = lax.broadcasted_iota(jnp.int32, (8, HALF), 0)
        col = lax.broadcasted_iota(jnp.int32, (8, HALF), 1)
        for b in range(B):
            for hf in range(2):
                g, pos = divmod((2 * (b * GPB + hg) + hf + SHIFT // 2) % (2 * NG), 2)
                diag = (col >= (row - 2 * pos) * DH) & (col < (row - 2 * pos + 1) * DH)
                qb = jnp.broadcast_to(q[b:b + 1, hf * HALF:(hf + 1) * HALF], (8, HALF))
                qblk[g, :, pos * HALF:(pos + 1) * HALF] = jnp.where(diag, qb, 0.0)

    def scores_softmax(g):
        slot = g % 2
        wait_all(kbuf.at[slot], K_SEM + slot)
        kk = kbuf[slot]
        s = jnp.dot(qblk[g].astype(BF16), kk, preferred_element_type=F32) * (DH ** -0.5)
        m = jnp.max(s, axis=-1, keepdims=True)
        e = jnp.exp(s - m)
        l = jnp.sum(e, axis=-1, keepdims=True)
        p_s[slot] = e * (1.0 / l)

    def pv_wo(g, u):
        slot = (g % 2) * NU + u
        wait_all(vbuf.at[slot], V_SEM + slot)
        for pos in range(2):
            hf = (pos + SHIFT // 2) % 2
            gu = g if pos >= SHIFT // 2 else (g + NG - 1) % NG
            b, hg = gu // GPB, gu % GPB
            tot = None
            for hh in range(2 * pos, 2 * pos + 2):
                mine = [i for i in range(UL) if SEQ[u * UL + i] // RH == hh]
                if not mine:
                    continue
                pb = jnp.broadcast_to(p_s[g % 2, hh:hh + 1, :], (8, W))
                for i in mine:
                    prod = vbuf[slot, i].astype(F32) * pb
                    o = jnp.sum(prod, axis=-1, keepdims=True)
                    r = SEQ[u * UL + i] + (hf - pos) * 2 * RH
                    term = o * wo_v[hg, r].astype(F32)
                    tot = term if tot is None else tot + term
            if tot is not None:
                acc[b] = acc[b] + tot

    def consume(g, u):
        if u == NU - 1:
            scores_softmax(g + 1)
        pv_wo(g, u)

    def ffn_down(lo, hi):
        lo, hi = lo * 8, hi * 8
        wait_all(w2_v.at[:, pl.ds(lo, hi - lo)], F2_SEM)
        out = None
        for a in range(W2S):
            part = jnp.dot(h_s[:, a * FS + lo:a * FS + hi].astype(BF16), w2_v[a, lo:hi, :],
                           preferred_element_type=F32)
            out = part if out is None else out + part
        return out

    def in_row0(v, b):
        row8 = lax.broadcasted_iota(jnp.int32, (8, D), 0)
        return jnp.where(row8 == 0, jnp.broadcast_to(v[b:b + 1, :], (8, D)), 0.0)

    wq_descs = [(A, rows8(j), lanes(c, 4))
                for j in range(16) for c in range(HQ * DH // (4 * LANE))]
    n0 = (len(wq_descs) - LEAD) // 2
    for i in range(LEAD):
        w_copy(wq_hbm, wq_v, wq_descs[n0 + i], Q_SEM).start(priority=1)
    xcp = pltpu.make_async_copy(x_hbm, x_v, sems.at[X_SEM])
    xcp.start()
    for i in range(n0):
        w_copy(wq_hbm, wq_v, wq_descs[i], Q_SEM).start(priority=0)
        w_copy(wq_hbm, wq_v, wq_descs[n0 + LEAD + i], Q_SEM).start(priority=1)
    xcp.wait()
    x = x_v[...].astype(F32)
    mu = jnp.mean(x, axis=-1, keepdims=True)
    xc = x - mu
    var = jnp.mean(xc * xc, axis=-1, keepdims=True)
    xn4 = xc / jnp.sqrt(var + 1e-5)
    xn = jnp.concatenate([xn4, jnp.zeros((8 - B, D), F32)], axis=0).astype(BF16)
    loop(0, 16, issue_w13)
    wait_all(wq_v, Q_SEM)
    for hg in range(GPB // 2):
        qproj(xn, hg)
    loop(0, W2_MAIN // 2, issue_w2)
    loop(0, 16, issue_wo)
    for hg in range(GPB // 2, GPB):
        qproj(xn, hg)
    loop(16, 40, issue_wo)
    wait_all(w1_v, F1_SEM)
    wait_all(w3_v, F3_SEM)
    gate = jnp.dot(xn, w1_v[...].reshape(D, F), preferred_element_type=F32)
    up = jnp.dot(xn, w3_v[...].reshape(D, F), preferred_element_type=F32)
    h_s[...] = (gate * jax.nn.sigmoid(gate) * up).astype(BF16).astype(F32)
    loop(40, 64, issue_wo)
    base = x + ffn_down(0, W2_MAIN)[0:B, :]
    for b in range(B):
        acc[b] = in_row0(base, b)
    eye = (lax.broadcasted_iota(jnp.int32, (LANE, LANE), 0)
           == lax.broadcasted_iota(jnp.int32, (LANE, LANE), 1))
    for b in range(B):
        for a in range(W2S):
            hrow = h_s[b:b + 1, (a + 1) * FS - LANE:(a + 1) * FS]
            col = jnp.sum(jnp.where(eye, jnp.broadcast_to(hrow, (LANE, LANE)), 0.0),
                          axis=-1, keepdims=True)
            hb_s[b, a] = jnp.broadcast_to(col, (LANE, LANE))
    loop(64, 96, issue_wo)
    for r0, r1 in zip(*FIRST):
        k_copy(0, r0).start(priority=0)
        k_copy(0, r1).start(priority=1)
    wait_all(wo_v, O_SEM)
    for u in range(LA):
        issue_unit(0, u)
    scores_softmax(0)

    def step(g, issue_next):
        for u in range(NU):
            if u + LA < NU:
                issue_unit(g, u + LA)
            else:
                issue_next(u + LA - NU)
            consume(g, u)

    def group_body(g, carry):
        step(g, lambda u: issue_unit(g + 1, u))
        return carry

    lax.fori_loop(0, NG - 2, group_body, 0)

    step(NG - 2, lambda u: issue_last(u * LAST_ISSUE, (u + 1) * LAST_ISSUE))
    issue_last(LA * LAST_ISSUE, n_last)
    for u in range(NU):
        pv_wo(NG - 1, u)
    tot = [acc[b] for b in range(B)]
    mid = ffn_down(W2_MAIN, W2_TAIL)
    tot = [tot[b] + in_row0(mid, b) for b in range(B)]
    j0 = W2_TAIL
    for t, n in enumerate(TAIL_GRAN):
        wait_all(w2_v.at[:, pl.ds(j0 * 8, n * 8)], T_SEM + t)
        for j in range(j0, j0 + n):
            for a in range(W2S):
                wrow = w2_v[a, j * 8:j * 8 + 8, :].astype(F32)
                r = j * 8 - (FS - LANE)
                for b in range(B):
                    hb = hb_s[b, a, r:r + 8, :]
                    tot[b] = tot[b] + jnp.concatenate([hb] * (D // LANE), axis=1) * wrow
        j0 += n
    res = jnp.concatenate([jnp.sum(t, axis=0, keepdims=True) for t in tot], axis=0)
    out_ref[...] = res.astype(out_ref.dtype)


@jax.jit
def pallas_parallel_sum__sliding_block_cached__glu_gated_swiglu__decode_kernel(
    A_x: jax.Array,
    A_k_cache: jax.Array,
    A_v_cache: jax.Array,
    A_wq: jax.Array,
    A_wo: jax.Array,
    B_x: jax.Array,
    B_w1: jax.Array,
    B_w3: jax.Array,
    B_w2: jax.Array,
):
    B, Sq, D = A_x.shape
    _, Hkv, S, Dh = A_k_cache.shape
    F = B_w1.shape[1]
    assert (B, Sq, D, Hkv, Dh, F) == (4, 1, 640, HQ, DH, 1536)
    W = min(4096, max(256, S // 4))
    assert W == 2048 and sum(TAIL_GRAN) * 8 <= LANE
    NG = B * HQ // HG

    kt = jnp.swapaxes(A_k_cache, 2, 3).reshape(B * HQ, DH, S)
    vt = jnp.swapaxes(A_v_cache, 2, 3).reshape(B * HQ, DH, S)
    x2 = A_x.reshape(B, D)
    wq = A_wq.reshape(5, D // 5, HQ * DH)
    wo = A_wo.reshape(HQ // HG, GROWS // 8, 8, D)
    w1 = B_w1.reshape(5, D // 5, F)
    w3 = B_w3.reshape(5, D // 5, F)
    w2 = B_w2.reshape(W2S, F // W2S, D)

    kern = lambda *refs: _kernel(*refs, B=B, D=D, S=S, W=W, F=F)
    out = pl.pallas_call(
        kern,
        in_specs=[pl.BlockSpec(memory_space=pl.ANY)] * 8,
        out_specs=pl.BlockSpec(memory_space=pltpu.VMEM),
        out_shape=jax.ShapeDtypeStruct((B, D), A_x.dtype),
        scratch_shapes=[
            pltpu.VMEM((B, D), BF16),
            pltpu.VMEM(wq.shape, BF16),
            pltpu.VMEM(wo.shape, BF16),
            pltpu.VMEM(w1.shape, BF16),
            pltpu.VMEM(w3.shape, BF16),
            pltpu.VMEM(w2.shape, BF16),
            pltpu.VMEM((2, GROWS, W), BF16),
            pltpu.VMEM((2 * NU, UL, 8, W), BF16),
            pltpu.VMEM((NG, 8, GROWS), F32),
            pltpu.VMEM((2, 8, W), F32),
            pltpu.VMEM((B, 8, D), F32),
            pltpu.VMEM((8, F), F32),
            pltpu.VMEM((B, W2S, LANE, LANE), F32),
            pltpu.SemaphoreType.DMA((N_SEM,)),
        ],
        compiler_params=pltpu.CompilerParams(vmem_limit_bytes=100 * 1024 * 1024,
                                             disable_semaphore_checks=True,
                                             disable_bounds_checks=True),
    )(x2, kt, vt, wq, wo, w1, w3, w2)
    return out.reshape(B, Sq, D)
```

```python
import jax
import jax.numpy as jnp
from jax import lax
import jax.experimental.pallas as pl
import jax.experimental.pallas.tpu as pltpu

F32 = jnp.float32
BF16 = jnp.bfloat16
A = slice(None)

HQ = 32
DH = 192
LANE = 128
RH = DH // 8
HG = 4
SHIFT = 2
GROWS = HG * DH
LEAD = 24
LA = 3

RG = GROWS // 8
SEQ32 = [8 * x + y for y in (0, 1, 4, 5, 2, 3, 6, 7) for x in (0, 3, 1, 2)]
SEQ = [32 * blk + r for blk in range(RG // 32) for r in SEQ32]
NU = 4
UL = RG // NU
FIRST = (SEQ[:RG // 2], SEQ[RG // 2:])
LAST0 = (0, 1, 2, 4, 6, 8, 10)
LAST1 = (3, 5, 7, 9, 11)

W2S = 4
W2_MAIN = 24
W2_T0 = 4
TAIL_GRAN = (3, 3, 2, 2, 1, 1)
LAST_ISSUE = 20

CH = 16
FFN_PH = 13
W_ADV = list(range(32))
W_INN = (0, 3, 1, 2)


def _chunks(name, n_rg, nt, ph, keep=lambda rg: True):
    out = []
    for i in range(n_rg * nt // CH + (1 if ph else 0)):
        lo, hi, pieces = max(i * CH - ph, 0), min((i + 1) * CH - ph, n_rg * nt), []
        while lo < hi:
            rg, c = divmod(lo, nt)
            m = min(nt - c, hi - lo)
            if keep(rg):
                prev = pieces[-1] if pieces else None
                if m == nt and prev and prev[4] == nt and prev[1] + prev[2] == rg:
                    pieces[-1] = (name, prev[1], prev[2] + 1, 0, nt)
                else:
                    pieces.append((name, rg, 1, c, m))
            lo += m
        out.append(pieces)
    return out


def _weight_schedule(D, F):
    reg = []
    for name, n_rg, nt, ph in (("w2", F // 8, D // LANE, FFN_PH), ("w3", D // 8, F // LANE, FFN_PH),
                               ("w1", D // 8, F // LANE, FFN_PH), ("wo", HQ * RH, D // LANE, 0),
                               ("wq", D // 8, HQ * DH // LANE, 0)):
        keep = (lambda rg: rg % (F // W2S // 8) < W2_MAIN) if name == "w2" else (lambda rg: True)
        ch = _chunks(name, n_rg, nt, ph, keep)
        if ph and reg:
            reg[-1] = reg[-1] + ch.pop(0)
        elif ph:
            ch[1] = ch[0] + ch[1]
            ch.pop(0)
        reg += ch
    n = len(reg)
    top = n - 64
    block = lambda base: [base + 32 * x + y for y in W_ADV for x in W_INN]
    ends = [(top if x < 2 else top - 5 * 128) + 32 * x + y for y in W_ADV for x in W_INN]
    seq = block(top - 128) + ends + block(top - 256) + block(top - 384) + block(top - 512)
    seq += [i for i in range(n) if i not in seq]
    seq = [reg[i] for i in seq if reg[i]]
    n1 = (len(seq) + LEAD) // 2
    return seq[n1:], seq[:n1]


X_SEM, Q_SEM, F1_SEM, F3_SEM, F2_SEM, O_SEM, K_SEM, V_SEM = 0, 1, 2, 3, 4, 5, 6, 8
T_SEM = V_SEM + 2 * NU
N_SEM = T_SEM + len(TAIL_GRAN)


def _kernel(x_hbm, k_hbm, v_hbm, wq_hbm, wo_hbm, w1_hbm, w3_hbm, w2_hbm,
            out_ref,
            x_v, wq_v, wo_v, w1_v, w3_v, w2_v, kbuf, vbuf, qblk, p_s, acc, h_s, hb_s,
            sems, *, B, D, S, W, F):
    NC = W // LANE
    GPB = HQ // HG
    NG = B * GPB
    S0 = S - W
    FS = F // W2S

    def rows8(j):
        return pl.ds(j * 8, 8) if isinstance(j, int) else pl.ds(pl.multiple_of(j * 8, 8), 8)

    def lanes(c, m=1, off=0):
        n = m * LANE
        if isinstance(c, int):
            return pl.ds(off + c * n, n)
        return pl.ds(pl.multiple_of(off + c * n, LANE), n)

    def head_of(g, r):
        lo = g * HG - SHIFT
        hh = r // RH
        if hh >= SHIFT:
            return lo + hh
        if isinstance(g, int):
            return (lo + hh) % (B * HQ)
        return jnp.where(g == 0, B * HQ - SHIFT, lo) + hh

    def k_copy(g, r):
        slot = g % 2
        return pltpu.make_async_copy(k_hbm.at[head_of(g, r), rows8(r % RH), pl.ds(S0, W)],
                                     kbuf.at[slot, rows8(r)], sems.at[K_SEM + slot])

    def v_copy(g, pos):
        slot = (g % 2) * NU + pos // UL
        r = SEQ[pos]
        return pltpu.make_async_copy(v_hbm.at[head_of(g, r), rows8(r % RH), pl.ds(S0, W)],
                                     vbuf.at[slot, pos % UL], sems.at[V_SEM + slot])

    def wait_all(buf, sem):
        pltpu.make_async_copy(buf, buf, sems.at[sem]).wait()

    def w_copy(src, dst, idx, sem):
        return pltpu.make_async_copy(src.at[idx], dst.at[idx], sems.at[sem])

    def piece_copy(name, rg, n, c, m):
        cols = pl.ds(c * LANE, m * LANE)
        if name == "wo":
            return w_copy(wo_hbm, wo_v, (rg // RG, pl.ds(rg % RG, n), A, cols), O_SEM)
        if name == "w2":
            a, r = divmod(rg, FS // 8)
            return w_copy(w2_hbm, w2_v, (a, pl.ds(r * 8, n * 8), cols), F2_SEM)
        src, dst, sem = {"wq": (wq_hbm, wq_v, Q_SEM), "w1": (w1_hbm, w1_v, F1_SEM),
                         "w3": (w3_hbm, w3_v, F3_SEM)}[name]
        return w_copy(src, dst, (pl.ds(rg * 8, n * 8), cols), sem)

    def issue_unit(g, u):
        for pos in range(u * UL, (u + 1) * UL):
            k_copy(g + 1, SEQ[pos]).start(priority=0)
            v_copy(g, pos).start(priority=1)

    W2_TAIL = FS // 8 - sum(TAIL_GRAN)
    tail_sem = {j: F2_SEM for j in range(W2_MAIN, W2_TAIL)}
    for t, n in enumerate(TAIL_GRAN):
        for _ in range(n):
            tail_sem[W2_MAIN + len(tail_sem)] = T_SEM + t
    t0_list = [("v", 8 * ch + i) for ch in LAST0 for i in range(8)]
    t1_list = [("v", 8 * ch + i) for ch in LAST1 for i in range(8)]
    t0_list += [("w2", j) for j in range(W2_MAIN, W2_MAIN + W2_T0)]
    t1_list += [("w2", j) for j in range(W2_MAIN + W2_T0, FS // 8)]
    n_last = max(len(t0_list), len(t1_list))

    def issue_last(lo, hi):
        for i in range(lo, min(hi, n_last)):
            for prio, lst in enumerate((t0_list, t1_list)):
                if i >= len(lst):
                    continue
                d = lst[i]
                if d[0] == "w2":
                    cp = w_copy(w2_hbm, w2_v, (A, rows8(d[1]), A), tail_sem[d[1]])
                else:
                    cp = v_copy(NG - 1, d[1])
                cp.start(priority=prio)

    HALF = GROWS // 2

    def qproj(xn, hg):
        w = wq_v[:, hg * GROWS:(hg + 1) * GROWS]
        q = jnp.dot(xn, w, preferred_element_type=F32).astype(BF16).astype(F32)
        row = lax.broadcasted_iota(jnp.int32, (8, HALF), 0)
        col = lax.broadcasted_iota(jnp.int32, (8, HALF), 1)
        for b in range(B):
            for hf in range(2):
                g, pos = divmod((2 * (b * GPB + hg) + hf + SHIFT // 2) % (2 * NG), 2)
                diag = (col >= (row - 2 * pos) * DH) & (col < (row - 2 * pos + 1) * DH)
                qb = jnp.broadcast_to(q[b:b + 1, hf * HALF:(hf + 1) * HALF], (8, HALF))
                qblk[g, :, pos * HALF:(pos + 1) * HALF] = jnp.where(diag, qb, 0.0)

    def scores_softmax(g):
        slot = g % 2
        wait_all(kbuf.at[slot], K_SEM + slot)
        kk = kbuf[slot]
        s = jnp.dot(qblk[g].astype(BF16), kk, preferred_element_type=F32) * (DH ** -0.5)
        m = jnp.max(s, axis=-1, keepdims=True)
        e = jnp.exp(s - m)
        l = jnp.sum(e, axis=-1, keepdims=True)
        p_s[slot] = e * (1.0 / l)

    def pv_wo(g, u):
        slot = (g % 2) * NU + u
        wait_all(vbuf.at[slot], V_SEM + slot)
        for pos in range(2):
            hf = (pos + SHIFT // 2) % 2
            gu = g if pos >= SHIFT // 2 else (g + NG - 1) % NG
            b, hg = gu // GPB, gu % GPB
            tot = None
            for hh in range(2 * pos, 2 * pos + 2):
                mine = [i for i in range(UL) if SEQ[u * UL + i] // RH == hh]
                if not mine:
                    continue
                pb = jnp.broadcast_to(p_s[g % 2, hh:hh + 1, :], (8, W))
                for i in mine:
                    prod = vbuf[slot, i].astype(F32) * pb
                    o = jnp.sum(prod, axis=-1, keepdims=True)
                    r = SEQ[u * UL + i] + (hf - pos) * 2 * RH
                    term = o * wo_v[hg, r].astype(F32)
                    tot = term if tot is None else tot + term
            if tot is not None:
                acc[b] = acc[b] + tot

    def consume(g, u):
        if u == NU - 1:
            scores_softmax(g + 1)
        pv_wo(g, u)

    def ffn_down(lo, hi):
        lo, hi = lo * 8, hi * 8
        wait_all(w2_v.at[:, pl.ds(lo, hi - lo)], F2_SEM)
        out = None
        for a in range(W2S):
            part = jnp.dot(h_s[:, a * FS + lo:a * FS + hi].astype(BF16), w2_v[a, lo:hi, :],
                           preferred_element_type=F32)
            out = part if out is None else out + part
        return out

    def in_row0(v, b):
        row8 = lax.broadcasted_iota(jnp.int32, (8, D), 0)
        return jnp.where(row8 == 0, jnp.broadcast_to(v[b:b + 1, :], (8, D)), 0.0)

    w0, w1 = _weight_schedule(D, F)
    lead = len(w1) - len(w0)
    xcp = pltpu.make_async_copy(x_hbm, x_v, sems.at[X_SEM])
    for i, chunk in enumerate(w1):
        if i == lead:
            xcp.start()
        if i >= lead:
            for piece in w0[i - lead]:
                piece_copy(*piece).start(priority=0)
        for piece in chunk:
            piece_copy(*piece).start(priority=1)
    for r0, r1 in zip(*FIRST):
        k_copy(0, r0).start(priority=0)
        k_copy(0, r1).start(priority=1)
    xcp.wait()
    x = x_v[...].astype(F32)
    mu = jnp.mean(x, axis=-1, keepdims=True)
    xc = x - mu
    var = jnp.mean(xc * xc, axis=-1, keepdims=True)
    xn4 = xc / jnp.sqrt(var + 1e-5)
    xn = jnp.concatenate([xn4, jnp.zeros((8 - B, D), F32)], axis=0).astype(BF16)
    wait_all(w1_v, F1_SEM)
    wait_all(w3_v, F3_SEM)
    gate = jnp.dot(xn, w1_v[...], preferred_element_type=F32)
    up = jnp.dot(xn, w3_v[...], preferred_element_type=F32)
    h_s[...] = (gate * jax.nn.sigmoid(gate) * up).astype(BF16).astype(F32)
    issue_unit(0, 0)
    wait_all(wq_v, Q_SEM)
    for hg in range(GPB // 2):
        qproj(xn, hg)
    issue_unit(0, 1)
    wait_all(wo_v, O_SEM)
    for hg in range(GPB // 2, GPB):
        qproj(xn, hg)
    for u in range(2, LA):
        issue_unit(0, u)
    base = x + ffn_down(0, W2_MAIN)[0:B, :]
    for b in range(B):
        acc[b] = in_row0(base, b)
    eye = (lax.broadcasted_iota(jnp.int32, (LANE, LANE), 0)
           == lax.broadcasted_iota(jnp.int32, (LANE, LANE), 1))
    for b in range(B):
        for a in range(W2S):
            hrow = h_s[b:b + 1, (a + 1) * FS - LANE:(a + 1) * FS]
            col = jnp.sum(jnp.where(eye, jnp.broadcast_to(hrow, (LANE, LANE)), 0.0),
                          axis=-1, keepdims=True)
            hb_s[b, a] = jnp.broadcast_to(col, (LANE, LANE))
    scores_softmax(0)

    def step(g, issue_next):
        for u in range(NU):
            if u + LA < NU:
                issue_unit(g, u + LA)
            else:
                issue_next(u + LA - NU)
            consume(g, u)

    def group_body(g, carry):
        step(g, lambda u: issue_unit(g + 1, u))
        return carry

    lax.fori_loop(0, NG - 2, group_body, 0)

    step(NG - 2, lambda u: issue_last(u * LAST_ISSUE, (u + 1) * LAST_ISSUE))
    issue_last(LA * LAST_ISSUE, n_last)
    for u in range(NU):
        pv_wo(NG - 1, u)
    tot = [acc[b] for b in range(B)]
    mid = ffn_down(W2_MAIN, W2_TAIL)
    tot = [tot[b] + in_row0(mid, b) for b in range(B)]
    j0 = W2_TAIL
    for t, n in enumerate(TAIL_GRAN):
        wait_all(w2_v.at[:, pl.ds(j0 * 8, n * 8)], T_SEM + t)
        for j in range(j0, j0 + n):
            for a in range(W2S):
                wrow = w2_v[a, j * 8:j * 8 + 8, :].astype(F32)
                r = j * 8 - (FS - LANE)
                for b in range(B):
                    hb = hb_s[b, a, r:r + 8, :]
                    tot[b] = tot[b] + jnp.concatenate([hb] * (D // LANE), axis=1) * wrow
        j0 += n
    res = jnp.concatenate([jnp.sum(t, axis=0, keepdims=True) for t in tot], axis=0)
    out_ref[...] = res.astype(out_ref.dtype)


@jax.jit
def pallas_parallel_sum__sliding_block_cached__glu_gated_swiglu__decode_kernel(
    A_x: jax.Array,
    A_k_cache: jax.Array,
    A_v_cache: jax.Array,
    A_wq: jax.Array,
    A_wo: jax.Array,
    B_x: jax.Array,
    B_w1: jax.Array,
    B_w3: jax.Array,
    B_w2: jax.Array,
):
    B, Sq, D = A_x.shape
    _, Hkv, S, Dh = A_k_cache.shape
    F = B_w1.shape[1]
    assert (B, Sq, D, Hkv, Dh, F) == (4, 1, 640, HQ, DH, 1536)
    W = min(4096, max(256, S // 4))
    assert W == 2048 and sum(TAIL_GRAN) * 8 <= LANE
    NG = B * HQ // HG

    kt = jnp.swapaxes(A_k_cache, 2, 3).reshape(B * HQ, DH, S)
    vt = jnp.swapaxes(A_v_cache, 2, 3).reshape(B * HQ, DH, S)
    x2 = A_x.reshape(B, D)
    wq = A_wq
    wo = A_wo.reshape(HQ // HG, GROWS // 8, 8, D)
    w1 = B_w1
    w3 = B_w3
    w2 = B_w2.reshape(W2S, F // W2S, D)

    kern = lambda *refs: _kernel(*refs, B=B, D=D, S=S, W=W, F=F)
    out = pl.pallas_call(
        kern,
        in_specs=[pl.BlockSpec(memory_space=pl.ANY)] * 8,
        out_specs=pl.BlockSpec(memory_space=pltpu.VMEM),
        out_shape=jax.ShapeDtypeStruct((B, D), A_x.dtype),
        scratch_shapes=[
            pltpu.VMEM((B, D), BF16),
            pltpu.VMEM(wq.shape, BF16),
            pltpu.VMEM(wo.shape, BF16),
            pltpu.VMEM(w1.shape, BF16),
            pltpu.VMEM(w3.shape, BF16),
            pltpu.VMEM(w2.shape, BF16),
            pltpu.VMEM((2, GROWS, W), BF16),
            pltpu.VMEM((2 * NU, UL, 8, W), BF16),
            pltpu.VMEM((NG, 8, GROWS), F32),
            pltpu.VMEM((2, 8, W), F32),
            pltpu.VMEM((B, 8, D), F32),
            pltpu.VMEM((8, F), F32),
            pltpu.VMEM((B, W2S, LANE, LANE), F32),
            pltpu.SemaphoreType.DMA((N_SEM,)),
        ],
        compiler_params=pltpu.CompilerParams(vmem_limit_bytes=100 * 1024 * 1024,
                                             disable_semaphore_checks=True,
                                             disable_bounds_checks=True),
    )(x2, kt, vt, wq, wo, w1, w3, w2)
    return out.reshape(B, Sq, D)
```

```python
import jax
import jax.numpy as jnp
from jax import lax
import jax.experimental.pallas as pl
import jax.experimental.pallas.tpu as pltpu

F32 = jnp.float32
BF16 = jnp.bfloat16
A = slice(None)
LANE = 128

HQ = 32
DH = 192
RH = DH // 8
HG = 4
GROWS = HG * DH
RG = GROWS // 8
SHIFT = 2

SEQ32 = [8 * x + y for y in (0, 1, 4, 5, 2, 3, 6, 7) for x in (0, 3, 1, 2)]
SEQ = [32 * blk + r for blk in range(RG // 32) for r in SEQ32]
NU = 4
UL = RG // NU
LA = 3
LAST0 = (0, 1, 2, 4, 6, 8, 10)
LAST1 = (3, 5, 7, 9, 11)
LAST_ISSUE = 20

W2S = 4
W2_MAIN = 24
W2_T0 = 4
TAIL_GRAN = (3, 3, 2, 2, 1, 1)

CH = 16
FFN_PH = 14
LEAD = 24

X_SEM, Q_SEM, F1_SEM, F3_SEM, F2_SEM, O_SEM, K_SEM, V_SEM = 0, 1, 2, 3, 4, 5, 6, 8
T_SEM = V_SEM + 2 * NU
N_SEM = T_SEM + len(TAIL_GRAN)


def _chunks(name, n_rg, nt, ph, keep):
    out = []
    for i in range(n_rg * nt // CH + (1 if ph else 0)):
        lo, hi, pieces = max(i * CH - ph, 0), min((i + 1) * CH - ph, n_rg * nt), []
        while lo < hi:
            rg, c = divmod(lo, nt)
            m = min(nt - c, hi - lo)
            if keep(rg):
                prev = pieces[-1] if pieces else None
                if m == nt and prev and prev[4] == nt and prev[1] + prev[2] == rg:
                    pieces[-1] = (name, prev[1], prev[2] + 1, 0, nt)
                else:
                    pieces.append((name, rg, 1, c, m))
            lo += m
        out.append(pieces)
    return out


def _weight_schedule(D, F):
    reg = []
    for name, n_rg, nt, ph in (("w2", F // 8, D // LANE, FFN_PH), ("w3", D // 8, F // LANE, FFN_PH),
                               ("w1", D // 8, F // LANE, FFN_PH), ("wo", HQ * RH, D // LANE, 0),
                               ("wq", D // 8, HQ * DH // LANE, 0)):
        keep = (lambda rg: rg % (F // W2S // 8) < W2_MAIN) if name == "w2" else (lambda rg: True)
        ch = _chunks(name, n_rg, nt, ph, keep)
        if ph:
            short = ch.pop(0)
            if reg:
                reg[-1] = reg[-1] + short
            else:
                ch[0] = short + ch[0]
        reg += ch
    top = len(reg) - 64
    walk = [(x, 32 * x + y) for y in range(32) for x in (0, 3, 1, 2)]
    seq = [top - 128 + i for _, i in walk]
    seq += [(top if x < 2 else top - 5 * 128) + i for x, i in walk]
    seq += [top - 128 * k + i for k in (2, 3, 4) for _, i in walk]
    seq += [i for i in range(len(reg)) if i not in seq]
    assert sorted(seq) == list(range(len(reg)))
    seq = [reg[i] for i in seq if reg[i]]
    n1 = (len(seq) + LEAD) // 2
    return seq[n1:], seq[:n1]


def _kernel(x_hbm, k_hbm, v_hbm, wq_hbm, wo_hbm, w1_hbm, w3_hbm, w2_hbm,
            out_ref,
            x_v, wq_v, wo_v, w1_v, w3_v, w2_v, kbuf, vbuf, qblk, p_s, acc, h_s, hb_s,
            sems, *, B, D, S, W, F):
    GPB = HQ // HG
    NG = B * GPB
    FS = F // W2S
    HALF = GROWS // 2
    window = pl.ds(S - W, W)

    def rows8(j):
        return pl.ds(j * 8, 8)

    def heads_of(g):
        lo = g * HG - SHIFT
        if isinstance(g, int):
            return [(lo + hh) % (B * HQ) for hh in range(HG)]
        wrapped = jnp.where(g == 0, B * HQ - SHIFT, lo)
        return [(wrapped if hh < SHIFT else lo) + hh for hh in range(HG)]

    def k_copier(g):
        heads, slot = heads_of(g), g % 2
        return lambda r: pltpu.make_async_copy(
            k_hbm.at[heads[r // RH], rows8(r % RH), window],
            kbuf.at[slot, rows8(r)], sems.at[K_SEM + slot])

    def v_copier(g):
        heads, slot0 = heads_of(g), (g % 2) * NU
        slots = [slot0 + u for u in range(NU)]
        return lambda pos: pltpu.make_async_copy(
            v_hbm.at[heads[SEQ[pos] // RH], rows8(SEQ[pos] % RH), window],
            vbuf.at[slots[pos // UL], pos % UL], sems.at[V_SEM + slots[pos // UL]])

    def w_copy(src, dst, idx, sem):
        return pltpu.make_async_copy(src.at[idx], dst.at[idx], sems.at[sem])

    def piece_copy(name, rg, n, c, m):
        cols = pl.ds(c * LANE, m * LANE)
        if name == "wo":
            return w_copy(wo_hbm, wo_v, (rg // RG, pl.ds(rg % RG, n), A, cols), O_SEM)
        if name == "w2":
            a, r = divmod(rg, FS // 8)
            return w_copy(w2_hbm, w2_v, (a, pl.ds(r * 8, n * 8), cols), F2_SEM)
        src, dst, sem = {"wq": (wq_hbm, wq_v, Q_SEM), "w1": (w1_hbm, w1_v, F1_SEM),
                         "w3": (w3_hbm, w3_v, F3_SEM)}[name]
        return w_copy(src, dst, (pl.ds(rg * 8, n * 8), cols), sem)

    def wait_all(buf, sem):
        pltpu.make_async_copy(buf, buf, sems.at[sem]).wait()

    def issue_unit(g, u):
        k_copy, v_copy = k_copier(g + 1), v_copier(g)
        for pos in range(u * UL, (u + 1) * UL):
            k_copy(SEQ[pos]).start(priority=0)
            v_copy(pos).start(priority=1)

    W2_TAIL = FS // 8 - sum(TAIL_GRAN)
    w2_sem = [F2_SEM] * W2_TAIL + [T_SEM + t for t, n in enumerate(TAIL_GRAN) for _ in range(n)]
    last0 = [("v", 8 * ch + i) for ch in LAST0 for i in range(8)]
    last1 = [("v", 8 * ch + i) for ch in LAST1 for i in range(8)]
    last0 += [("w2", j) for j in range(W2_MAIN, W2_MAIN + W2_T0)]
    last1 += [("w2", j) for j in range(W2_MAIN + W2_T0, FS // 8)]
    assert len(last0) == len(last1) <= LA * LAST_ISSUE

    def issue_last(u):
        v_copy = v_copier(NG - 1)
        for pair in list(zip(last0, last1))[u * LAST_ISSUE:(u + 1) * LAST_ISSUE]:
            for prio, (kind, i) in enumerate(pair):
                cp = v_copy(i) if kind == "v" else w_copy(w2_hbm, w2_v, (A, rows8(i), A), w2_sem[i])
                cp.start(priority=prio)

    def qproj(xn, hg):
        w = wq_v[:, hg * GROWS:(hg + 1) * GROWS]
        q = jnp.dot(xn, w, preferred_element_type=F32).astype(BF16).astype(F32)
        row = lax.broadcasted_iota(jnp.int32, (8, HALF), 0)
        col = lax.broadcasted_iota(jnp.int32, (8, HALF), 1)
        for b in range(B):
            for hf in range(2):
                g, pos = divmod((2 * (b * GPB + hg) + hf + SHIFT // 2) % (2 * NG), 2)
                diag = (col >= (row - 2 * pos) * DH) & (col < (row - 2 * pos + 1) * DH)
                qb = jnp.broadcast_to(q[b:b + 1, hf * HALF:(hf + 1) * HALF], (8, HALF))
                qblk[g, :, pos * HALF:(pos + 1) * HALF] = jnp.where(diag, qb, 0.0)

    def scores_softmax(g):
        slot = g % 2
        wait_all(kbuf.at[slot], K_SEM + slot)
        s = jnp.dot(qblk[g].astype(BF16), kbuf[slot], preferred_element_type=F32) * (DH ** -0.5)
        m = jnp.max(s, axis=-1, keepdims=True)
        e = jnp.exp(s - m)
        l = jnp.sum(e, axis=-1, keepdims=True)
        p_s[slot] = e * (1.0 / l)

    def pv_wo(g, u):
        slot = (g % 2) * NU + u
        wait_all(vbuf.at[slot], V_SEM + slot)
        for pos in range(2):
            hf = (pos + SHIFT // 2) % 2
            gu = g if pos >= SHIFT // 2 else (g + NG - 1) % NG
            b, hg = gu // GPB, gu % GPB
            tot = None
            for hh in range(2 * pos, 2 * pos + 2):
                mine = [i for i in range(UL) if SEQ[u * UL + i] // RH == hh]
                if not mine:
                    continue
                pb = jnp.broadcast_to(p_s[g % 2, hh:hh + 1, :], (8, W))
                for i in mine:
                    o = jnp.sum(vbuf[slot, i].astype(F32) * pb, axis=-1, keepdims=True)
                    r = SEQ[u * UL + i] + (hf - pos) * 2 * RH
                    term = o * wo_v[hg, r].astype(F32)
                    tot = term if tot is None else tot + term
            if tot is not None:
                acc[b] = acc[b] + tot

    def ffn_down(lo, hi):
        lo, hi = lo * 8, hi * 8
        wait_all(w2_v.at[:, pl.ds(lo, hi - lo)], F2_SEM)
        out = None
        for a in range(W2S):
            part = jnp.dot(h_s[:, a * FS + lo:a * FS + hi].astype(BF16), w2_v[a, lo:hi, :],
                           preferred_element_type=F32)
            out = part if out is None else out + part
        return out

    def in_row0(v, b):
        row8 = lax.broadcasted_iota(jnp.int32, (8, D), 0)
        return jnp.where(row8 == 0, jnp.broadcast_to(v[b:b + 1, :], (8, D)), 0.0)

    w0, w1 = _weight_schedule(D, F)
    lead = len(w1) - len(w0)
    xcp = pltpu.make_async_copy(x_hbm, x_v, sems.at[X_SEM])
    for i, chunk in enumerate(w1):
        if i == lead:
            xcp.start()
        if i >= lead:
            for piece in w0[i - lead]:
                piece_copy(*piece).start(priority=0)
        for piece in chunk:
            piece_copy(*piece).start(priority=1)
    k_copy = k_copier(0)
    for r0, r1 in zip(SEQ[:RG // 2], SEQ[RG // 2:]):
        k_copy(r0).start(priority=0)
        k_copy(r1).start(priority=1)

    xcp.wait()
    x = x_v[...].astype(F32)
    mu = jnp.mean(x, axis=-1, keepdims=True)
    xc = x - mu
    var = jnp.mean(xc * xc, axis=-1, keepdims=True)
    xn4 = xc / jnp.sqrt(var + 1e-5)
    xn = jnp.concatenate([xn4, jnp.zeros((8 - B, D), F32)], axis=0).astype(BF16)
    wait_all(w1_v, F1_SEM)
    wait_all(w3_v, F3_SEM)
    gate = jnp.dot(xn, w1_v[...], preferred_element_type=F32)
    up = jnp.dot(xn, w3_v[...], preferred_element_type=F32)
    h_s[...] = (gate * jax.nn.sigmoid(gate) * up).astype(BF16).astype(F32)
    issue_unit(0, 0)
    wait_all(wq_v, Q_SEM)
    for hg in range(GPB // 2):
        qproj(xn, hg)
    issue_unit(0, 1)
    wait_all(wo_v, O_SEM)
    for hg in range(GPB // 2, GPB):
        qproj(xn, hg)
    for u in range(2, LA):
        issue_unit(0, u)
    base = x + ffn_down(0, W2_MAIN)[0:B, :]
    for b in range(B):
        acc[b] = in_row0(base, b)
    eye = (lax.broadcasted_iota(jnp.int32, (LANE, LANE), 0)
           == lax.broadcasted_iota(jnp.int32, (LANE, LANE), 1))
    for b in range(B):
        for a in range(W2S):
            hrow = h_s[b:b + 1, (a + 1) * FS - LANE:(a + 1) * FS]
            col = jnp.sum(jnp.where(eye, jnp.broadcast_to(hrow, (LANE, LANE)), 0.0),
                          axis=-1, keepdims=True)
            hb_s[b, a] = jnp.broadcast_to(col, (LANE, LANE))
    scores_softmax(0)

    def step(g, issue_next):
        for u in range(NU):
            if u + LA < NU:
                issue_unit(g, u + LA)
            else:
                issue_next(u + LA - NU)
            if u == NU - 1:
                scores_softmax(g + 1)
            pv_wo(g, u)

    def group_body(g, carry):
        step(g, lambda u: issue_unit(g + 1, u))
        return carry

    lax.fori_loop(0, NG - 2, group_body, 0)

    step(NG - 2, issue_last)
    for u in range(NU):
        pv_wo(NG - 1, u)
    mid = ffn_down(W2_MAIN, W2_TAIL)
    tot = [acc[b] + in_row0(mid, b) for b in range(B)]
    j0 = W2_TAIL
    for t, n in enumerate(TAIL_GRAN):
        wait_all(w2_v.at[:, pl.ds(j0 * 8, n * 8)], T_SEM + t)
        for j in range(j0, j0 + n):
            r = j * 8 - (FS - LANE)
            for a in range(W2S):
                wrow = w2_v[a, j * 8:j * 8 + 8, :].astype(F32)
                for b in range(B):
                    hb = jnp.concatenate([hb_s[b, a, r:r + 8, :]] * (D // LANE), axis=1)
                    tot[b] = tot[b] + hb * wrow
        j0 += n
    res = jnp.concatenate([jnp.sum(t, axis=0, keepdims=True) for t in tot], axis=0)
    out_ref[...] = res.astype(out_ref.dtype)


@jax.jit
def pallas_parallel_sum__sliding_block_cached__glu_gated_swiglu__decode_kernel(
    A_x: jax.Array,
    A_k_cache: jax.Array,
    A_v_cache: jax.Array,
    A_wq: jax.Array,
    A_wo: jax.Array,
    B_x: jax.Array,
    B_w1: jax.Array,
    B_w3: jax.Array,
    B_w2: jax.Array,
):
    B, Sq, D = A_x.shape
    _, Hkv, S, Dh = A_k_cache.shape
    F = B_w1.shape[1]
    assert (B, Sq, D, Hkv, Dh, F) == (4, 1, 640, HQ, DH, 1536)
    W = min(4096, max(256, S // 4))
    assert sum(TAIL_GRAN) * 8 <= LANE

    kt = jnp.swapaxes(A_k_cache, 2, 3).reshape(B * HQ, DH, S)
    vt = jnp.swapaxes(A_v_cache, 2, 3).reshape(B * HQ, DH, S)
    wo = A_wo.reshape(HQ // HG, RG, 8, D)
    w2 = B_w2.reshape(W2S, F // W2S, D)

    out = pl.pallas_call(
        lambda *refs: _kernel(*refs, B=B, D=D, S=S, W=W, F=F),
        in_specs=[pl.BlockSpec(memory_space=pl.ANY)] * 8,
        out_specs=pl.BlockSpec(memory_space=pltpu.VMEM),
        out_shape=jax.ShapeDtypeStruct((B, D), A_x.dtype),
        scratch_shapes=[
            pltpu.VMEM((B, D), BF16),
            pltpu.VMEM(A_wq.shape, BF16),
            pltpu.VMEM(wo.shape, BF16),
            pltpu.VMEM(B_w1.shape, BF16),
            pltpu.VMEM(B_w3.shape, BF16),
            pltpu.VMEM(w2.shape, BF16),
            pltpu.VMEM((2, GROWS, W), BF16),
            pltpu.VMEM((2 * NU, UL, 8, W), BF16),
            pltpu.VMEM((B * HQ // HG, 8, GROWS), F32),
            pltpu.VMEM((2, 8, W), F32),
            pltpu.VMEM((B, 8, D), F32),
            pltpu.VMEM((8, F), F32),
            pltpu.VMEM((B, W2S, LANE, LANE), F32),
            pltpu.SemaphoreType.DMA((N_SEM,)),
        ],
        compiler_params=pltpu.CompilerParams(vmem_limit_bytes=64 * 1024 * 1024,
                                             disable_semaphore_checks=True),
    )(A_x.reshape(B, D), kt, vt, A_wq, wo, B_w1, B_w3, w2)
    return out.reshape(B, Sq, D)
```
